```python
import os as _os
_os.environ.setdefault("JAX_PLATFORMS", "cpu")
import jax
import jax.numpy as jnp

def _softmax(x, axis=-1):
    return jax.nn.softmax(x, axis=axis)
def _gelu(x):
    return jax.nn.gelu(x, approximate=True)
def _silu(x):
    return jax.nn.silu(x)
def _sigmoid(x):
    return jax.nn.sigmoid(x)
def _layernorm(x, axis=-1, eps=1e-5):
    m = jnp.mean(x, axis=axis, keepdims=True)
    v = jnp.var(x, axis=axis, keepdims=True)
    return (x - m) / jnp.sqrt(v + eps)
def _scatter_add(tgt, idx, src, axis=0):
    return tgt.at[idx].add(src)
def _segment_sum(src, seg, n):
    return jax.ops.segment_sum(src, seg, n)
class _Rng:
    def __init__(self, key):
        self._k = key
    def _next(self):
        self._k, sub = jax.random.split(self._k)
        return sub
    def normal(self, shape):
        return jax.random.normal(self._next(), shape, dtype=jnp.bfloat16)
    def randint(self, lo, hi, shape):
        return jax.random.randint(self._next(), shape, lo, hi, dtype=jnp.int32)
    def uniform(self, shape, lo=0.0, hi=1.0):
        return jax.random.uniform(self._next(), shape, jnp.bfloat16, lo, hi)
    def permutation(self, n):
        return jax.random.permutation(self._next(), n)


kernel_name = 'standalone__mha_softmax__prompt'

def setup_inputs():
    _rng = _Rng(jax.random.key(int.from_bytes(__import__("os").urandom(4), "little")))
    _w = (lambda a: (lambda t: t.astype(jnp.bfloat16) if jnp.issubdtype(t.dtype, jnp.floating) else t)(jnp.asarray(a)))
    B, H, Sq, Sk, D = 1, 32, 2048, 2048, 192
    return {
        "q": _w((lambda *s: _rng.normal(s) * 0.4)(B, H, Sq, D)),
        "k": _w((lambda *s: _rng.normal(s) * 0.4)(B, H, Sk, D)),
        "v": _w((lambda *s: _rng.normal(s) * 0.05)(B, H, Sk, D)),
    }

def reference(q, k, v):
    scale = q.shape[-1] ** -0.5
    scores = jnp.einsum("bhqd,bhkd->bhqk", q, k) * scale
    p = _softmax(scores, axis=-1)
    return jnp.einsum("bhqk,bhkd->bhqd", p, v)
```

```python
import functools, math
import jax, jax.numpy as jnp
from jax import lax
import jax.experimental.pallas as pl
import jax.experimental.pallas.tpu as pltpu

f32 = jnp.float32; bf16 = jnp.bfloat16

@jax.jit
def pallas_standalone__mha_softmax__prompt_kernel(q, k, v):
    r=128; g=2; w=256; dyn=False; upi=2; order='qk_first'; nbuf=2; lead=0
    B, H, S, D = q.shape
    qt = jnp.swapaxes(q, 2, 3).reshape(H, D, S)
    kt = jnp.swapaxes(k, 2, 3).reshape(H, D, S)
    vt = jnp.swapaxes(v, 2, 3).reshape(H, D, S)
    c = (D ** -0.5) * math.log2(math.e)
    half = S // 2
    NU = S // w
    nqc = half // r
    npv = S // (128 * g)

    def body(qt_ref, qn_ref, k0_ref, kn_ref, vt_ref, ot_ref, a_scr, m_scr, *sbufs):
        h = pl.program_id(0)
        z = pl.multiple_of(lax.shift_right_logical(h, 16) * 8, 8) if dyn else 0

        def col(u):
            if isinstance(u, int):
                return pl.ds(u * w, w)
            return pl.ds(pl.multiple_of(u * w, w), w)

        def srows(start, n):
            return pl.ds(pl.multiple_of(z + start, 8), n) if dyn else pl.ds(start, n)

        def prep_gen(kt_ref):
            for ci in range(nqc):
                c1 = pl.ds(ci * r, r); c2 = pl.ds(half + ci * r, r)
                k1 = kt_ref[:, c1].astype(f32); k2 = kt_ref[:, c2].astype(f32)
                a1t = jnp.concatenate([k1[0:64], k1[64:128] - k2[64:128]], axis=0)
                a2t = jnp.concatenate([k2[0:64], k2[128:192] - k1[128:192]], axis=0)
                a3t = jnp.concatenate([k2[64:128], k1[128:192]], axis=0)
                a_scr[0, c1, :] = a1t.T.astype(bf16)
                a_scr[1, c1, :] = a2t.T.astype(bf16)
                a_scr[2, c1, :] = a3t.T.astype(bf16)
                yield

        def qk_gen(qc, s_ref, res):
            w1 = qc[0:128]
            w2 = jnp.concatenate([qc[0:64], qc[128:192]], axis=0)
            w3 = qc[64:192]
            mx = None
            for ci in range(nqc):
                rows = pl.ds(ci * r, r)
                m3 = jnp.dot(a_scr[2, rows, :], w3, preferred_element_type=f32)
                m1 = jnp.dot(a_scr[0, rows, :], w1, preferred_element_type=f32)
                m2 = jnp.dot(a_scr[1, rows, :], w2, preferred_element_type=f32)
                s1 = m1 + m3
                s2 = m2 + m3
                s_ref[srows(ci * r, r), :] = s1
                s_ref[srows(half + ci * r, r), :] = s2
                t = jnp.maximum(s1, s2).reshape(r // 8, 8, w).max(axis=0)
                mx = t if mx is None else jnp.maximum(mx, t)
                yield
            res.append(jnp.max(mx, axis=0, keepdims=True))

        def smpv_gen(u, s_ref, m):
            acc = None; l = None
            for j in range(npv):
                ks = pl.ds(j * 128 * g, 128 * g)
                p = jnp.exp2((s_ref[srows(j * 128 * g, 128 * g), :] - m) * c)
                t = p.reshape(16 * g, 8, w).sum(axis=0)
                l = t if l is None else l + t
                o = jnp.dot(vt_ref[:, ks], p.astype(bf16), preferred_element_type=f32)
                acc = o if acc is None else acc + o
                yield
            lsum = jnp.sum(l, axis=0, keepdims=True)
            ot_ref[:, col(u)] = (acc * (1.0 / lsum)).astype(bf16)

        def run(*gens):
            gens = list(gens)
            alive = [True] * len(gens)
            while any(alive):
                for i, gg in enumerate(gens):
                    if alive[i]:
                        try: next(gg)
                        except StopIteration: alive[i] = False

        def fused(qc, s_w, u_sm, s_r, m, extra=()):
            res = []
            ga = qk_gen(qc, s_w, res); gb = smpv_gen(u_sm, s_r, m)
            for _ in range(lead):
                next(ga)
                for e in extra: next(e)
            if order == 'qk_first': run(ga, *extra, gb)
            else: run(gb, ga, *extra)
            return res[0]

        @pl.when(h == 0)
        def _():
            res = []
            run(prep_gen(k0_ref))
            run(qk_gen(qt_ref[:, col(0)], sbufs[0], res))
            m_scr[...] = res[0]

        m = m_scr[...]
        start = 0
        if upi:
            nit = (NU - 2) // upi
            def it(i, m):
                for uu in range(upi):
                    u = i * upi + uu
                    m = fused(qt_ref[:, col(u + 1)], sbufs[(uu + 1) % nbuf], u, sbufs[uu % nbuf], m)
                return m
            m = lax.fori_loop(0, nit, it, m)
            start = nit * upi
        for u in range(start, NU - 1):
            extra = (prep_gen(kn_ref),) if u == NU - 2 else ()
            m = fused(qt_ref[:, col(u + 1)], sbufs[(u + 1) % nbuf], u, sbufs[u % nbuf], m, extra)
        m = fused(qn_ref[...], sbufs[0], NU - 1, sbufs[(NU - 1) % nbuf], m)
        m_scr[...] = m

    nxt = lambda h: jnp.minimum(h + 1, H - 1)
    ot = pl.pallas_call(
        body,
        grid=(H,),
        in_specs=[
            pl.BlockSpec((None, D, S), lambda h: (h, 0, 0)),
            pl.BlockSpec((None, D, w), lambda h: (nxt(h), 0, 0)),
            pl.BlockSpec((None, D, S), lambda h: (0, 0, 0)),
            pl.BlockSpec((None, D, S), lambda h: (nxt(h), 0, 0)),
            pl.BlockSpec((None, D, S), lambda h: (h, 0, 0)),
        ],
        out_specs=pl.BlockSpec((None, D, S), lambda h: (h, 0, 0)),
        out_shape=jax.ShapeDtypeStruct((H, D, S), bf16),
        scratch_shapes=[pltpu.VMEM((3, half, 128), bf16), pltpu.VMEM((1, w), f32)] + [pltpu.VMEM((S, w), f32)] * nbuf,
        compiler_params=pltpu.CompilerParams(
            dimension_semantics=("arbitrary",),
            vmem_limit_bytes=100 * 1024 * 1024),
    )(qt, qt, kt, kt, vt)
    return jnp.swapaxes(ot.reshape(B, H, D, S), 2, 3)
```

```python
import functools, math
import jax, jax.numpy as jnp
from jax import lax
import jax.experimental.pallas as pl
import jax.experimental.pallas.tpu as pltpu

f32 = jnp.float32; bf16 = jnp.bfloat16; i32 = jnp.int32; u32 = jnp.uint32

@jax.jit
def pallas_standalone__mha_softmax__prompt_kernel(q, k, v):
    r=128; kc=256; pw=256; w=256; lead=0; pin=1; pinlag=1; premul=1; nobc=0; ploop=1
    B, H, S, D = q.shape
    qt = jnp.swapaxes(q, 2, 3).reshape(H, D, S)
    kt = jnp.swapaxes(k, 2, 3).reshape(H, D, S)
    vt = jnp.swapaxes(v, 2, 3).reshape(H, D, S)
    c = (D ** -0.5) * math.log2(math.e)
    half = S // 2
    NU = S // w
    nqc = half // r
    nkc = S // kc
    npv = nkc * (w // pw)
    QI, KI, VI = 0, 1, 2

    def body(q_hbm, k_hbm, v_hbm, o_hbm, inb, outb, a_scr, s0, s1, in_sem, out_sem, p_sem):
        sbufs = (s0, s1)
        zv = [None]
        def set_z(i):
            z0 = lax.shift_right_logical(i, 16)
            zv[0] = jnp.full((8, pw), z0, i32)
            return z0

        def in_copies(h, slot):
            return [pltpu.make_async_copy(src.at[h], inb.at[slot, i], in_sem.at[slot])
                    for i, src in ((KI, k_hbm), (QI, q_hbm), (VI, v_hbm))]

        def in_wait(slot):
            pltpu.make_async_copy(inb.at[slot], inb.at[slot], in_sem.at[slot]).wait()

        def out_copy(h, slot):
            return pltpu.make_async_copy(outb.at[slot], o_hbm.at[h], out_sem.at[slot])

        def tred(x, op):
            parts = [x[i * 8:(i + 1) * 8] for i in range(x.shape[0] // 8)]
            while len(parts) > 1:
                parts = [op(parts[i], parts[i + 1]) for i in range(0, len(parts), 2)]
            return parts[0]

        def a_store(i, ci, x):
            a_scr[i, pl.ds(ci * r // 2, r // 2), :] = pltpu.bitcast(x.astype(bf16), u32)

        def a_load(i, ci):
            return pltpu.bitcast(a_scr[i, pl.ds(ci * r // 2, r // 2), :], bf16)

        def prep_chunk(slot, ci):
            c1 = pl.ds(ci * r, r); c2 = pl.ds(half + ci * r, r)
            k1 = inb[slot, KI, :, c1].astype(f32); k2 = inb[slot, KI, :, c2].astype(f32)
            a1t = jnp.concatenate([k1[0:64], k1[64:128] - k2[64:128]], axis=0)
            a2t = jnp.concatenate([k2[0:64], k2[128:192] - k1[128:192]], axis=0)
            a3t = jnp.concatenate([k2[64:128], k1[128:192]], axis=0)
            a_store(0, ci, a1t.T); a_store(1, ci, a2t.T); a_store(2, ci, a3t.T)

        def cols(u, off=0, n=w):
            if isinstance(u, int):
                return pl.ds(u * w + off, n)
            return pl.ds(pl.multiple_of(u * w + off, 128), n)

        def weights(slot, u):
            qc = inb[slot, QI, :, cols(u)]
            return (qc[0:128], jnp.concatenate([qc[0:64], qc[128:192]], axis=0), qc[64:192])

        def qk_chunk(ws, s_ref, ci, mx):
            w1, w2, w3 = ws
            m3 = jnp.dot(a_load(2, ci), w3, preferred_element_type=f32)
            m1 = jnp.dot(a_load(0, ci), w1, preferred_element_type=f32)
            m2 = jnp.dot(a_load(1, ci), w2, preferred_element_type=f32)
            s1_ = m1 + m3
            s2_ = m2 + m3
            if premul:
                s1_ = s1_ * c; s2_ = s2_ * c
            s_ref[pl.ds(ci * r, r), :] = s1_
            s_ref[pl.ds(half + ci * r, r), :] = s2_
            t = jnp.maximum(s1_, s2_).reshape(r // 8, 8, w).max(axis=0)
            return t if mx is None else jnp.maximum(mx, t)

        def fin_max(mx):
            return jnp.broadcast_to(jnp.max(mx, axis=0, keepdims=True), (8, w))

        def sm_chunk(slot, s_ref, kj, cj, m8, acc, l):
            ks = pl.ds(kj * kc, kc)
            s = s_ref[ks, pl.ds(cj * pw, pw)].reshape(kc // 8, 8, pw)
            x = s - m8[None]
            if not premul: x = x * c
            p = jnp.exp2(x).reshape(kc, pw)
            t = tred(p, jnp.add)
            l = t if l is None else l + t
            o = jnp.dot(inb[slot, VI, :, ks], p.astype(bf16), preferred_element_type=f32)
            acc = o if acc is None else acc + o
            return acc, l

        def dep(x, y):
            xb = lax.bitcast_convert_type(x, i32); yb = lax.bitcast_convert_type(y, i32)
            return lax.bitcast_convert_type(xb | (yb & zv[0]), f32)

        def fused(qk, sm, m8, prep=None):
            events = []
            if qk is not None:
                ws = weights(qk[0], qk[1])
                events += [(ci * npv, 0, ci) for ci in range(nqc)]
            if sm is not None:
                events += [((j * nqc + lead * npv), 1, j) for j in range(npv)]
            events.sort()
            mx = None; acc = None; l = None
            mxs = []
            for _, kind, idx in events:
                if kind == 0:
                    mx = qk_chunk(ws, sbufs[qk[2]], idx, mx)
                    mxs.append(mx)
                    if prep is not None: prep_chunk(prep, idx)
                else:
                    cj, kj = divmod(idx, nkc)
                    if kj == 0: acc = None; l = None
                    pj = len(mxs) - 2 - pinlag
                    mm = m8[:, cj * pw:(cj + 1) * pw]
                    if pin and pj >= 0 and zv[0] is not None: mm = dep(mm, mxs[pj][:, 0:pw])
                    acc, l = sm_chunk(sm[0], sbufs[sm[2]], kj, cj, mm, acc, l)
                    if kj == nkc - 1:
                        lsum = jnp.sum(l, axis=0, keepdims=True)
                        outb[sm[0], :, cols(sm[1], cj * pw, pw)] = (acc * (1.0 / lsum)).astype(bf16)
            return fin_max(mx) if qk is not None else None

        ck = pltpu.make_async_copy(k_hbm.at[0], inb.at[0, KI], p_sem.at[0])
        cq = pltpu.make_async_copy(q_hbm.at[0], inb.at[0, QI], p_sem.at[1])
        cv = pltpu.make_async_copy(v_hbm.at[0], inb.at[0, VI], p_sem.at[2])
        ck.start(); cq.start(); cv.start()
        for cp in in_copies(1, 1): cp.start()
        ck.wait(); cq.wait()
        ws = weights(0, 0)
        mx = None
        for ci in range(nqc):
            prep_chunk(0, ci)
            mx = qk_chunk(ws, sbufs[0], ci, mx)
        m = fin_max(mx)
        cv.wait()
        if ploop:
            def pit(i, m):
                u = 2 * i
                z0 = set_z(i)
                s1[pl.ds(pl.multiple_of(z0 * 8, 8), 8), :] = jnp.zeros((8, w), f32)
                m = fused((0, u + 1, 1), (0, u, 0), m)
                m = fused((0, u + 2, 0), (0, u + 1, 1), m)
                return m
            m = lax.fori_loop(0, (NU - 2) // 2, pit, m)
        else:
            for u in range(NU - 2):
                m = fused((0, u + 1, (u + 1) % 2), (0, u, u % 2), m)

        def step(h, m):
            cur = lax.rem(h, 2); nx = 1 - cur
            set_z(h)
            in_wait(nx)
            @pl.when(h > 0)
            def _():
                out_copy(h - 1, nx).wait()
            m = fused((cur, NU - 1, (NU - 1) % 2), (cur, NU - 2, (NU - 2) % 2), m, prep=nx)
            m = fused((nx, 0, 0), (cur, NU - 1, (NU - 1) % 2), m)
            out_copy(h, cur).start()
            hn = jnp.minimum(h + 2, H - 1)
            for cp in in_copies(hn, cur): cp.start()
            for u in range(NU - 2):
                m = fused((nx, u + 1, (u + 1) % 2), (nx, u, u % 2), m)
            return m
        m = lax.fori_loop(0, H - 1, step, m)

        last = (H - 1) % 2
        zv[0] = None
        e0 = pltpu.make_async_copy(outb.at[last, :, pl.ds(0, (NU - 2) * w)], o_hbm.at[H - 1, :, pl.ds(0, (NU - 2) * w)], p_sem.at[0])
        e1 = pltpu.make_async_copy(outb.at[last, :, pl.ds((NU - 2) * w, w)], o_hbm.at[H - 1, :, pl.ds((NU - 2) * w, w)], p_sem.at[1])
        e2 = pltpu.make_async_copy(outb.at[last, :, pl.ds((NU - 1) * w, w)], o_hbm.at[H - 1, :, pl.ds((NU - 1) * w, w)], p_sem.at[2])
        e0.start()
        m = fused((last, NU - 1, (NU - 1) % 2), (last, NU - 2, (NU - 2) % 2), m)
        e1.start()
        fused(None, (last, NU - 1, (NU - 1) % 2), m)
        e2.start()
        in_wait(1 - last)
        out_copy(H - 2, 1 - last).wait()
        e0.wait(); e1.wait(); e2.wait()

    ot = pl.pallas_call(
        body,
        in_specs=[pl.BlockSpec(memory_space=pl.ANY)] * 3,
        out_specs=pl.BlockSpec(memory_space=pl.ANY),
        out_shape=jax.ShapeDtypeStruct((H, D, S), bf16),
        scratch_shapes=[
            pltpu.VMEM((2, 3, D, S), bf16), pltpu.VMEM((2, D, S), bf16),
            pltpu.VMEM((3, half // 2, 128), u32), pltpu.VMEM((S, w), f32), pltpu.VMEM((S, w), f32),
            pltpu.SemaphoreType.DMA((2,)), pltpu.SemaphoreType.DMA((2,)), pltpu.SemaphoreType.DMA((3,)),
        ],
        compiler_params=pltpu.CompilerParams(
            vmem_limit_bytes=100 * 1024 * 1024, disable_bounds_checks=bool(nobc)),
    )(qt, kt, vt)
    return jnp.swapaxes(ot.reshape(B, H, D, S), 2, 3)
```

```python
import functools, math
import jax, jax.numpy as jnp
from jax import lax
import jax.experimental.pallas as pl
import jax.experimental.pallas.tpu as pltpu

f32 = jnp.float32; bf16 = jnp.bfloat16; i32 = jnp.int32; u32 = jnp.uint32

@jax.jit
def pallas_standalone__mha_softmax__prompt_kernel(q, k, v):
    premul=1; nobc=0; ksplit=2; bal=1; slab=16; porder='1302456'; ylag=5; slag=4; pace=1; plag=0; noprep=0
    klag=6; ppos=1; clag=0; f3=1; gate=1; kgap=3; vgap=1; zmode=1; etile=1
    B, H, S, D = q.shape
    qt = jnp.swapaxes(q, 2, 3).reshape(H, D, S)
    kt = jnp.swapaxes(k, 2, 3).reshape(H, D, S)
    vt = jnp.swapaxes(v, 2, 3).reshape(H, D, S)
    c = (D ** -0.5) * math.log2(math.e)
    w = 256; r = 128; hd = D // 2
    half = S // 2
    NU = S // w
    NC = S // (2 * r)
    QI, KI, VI = 0, 1, 2
    porder_ = [int(x) for x in str(porder).zfill(7)]
    SPC = r // slab
    SPT = SPC // 2

    def body(q_hbm, k_hbm, v_hbm, o_hbm, inb, outb, a_scr, x_scr, an_scr, xn_scr, s0, s1, y0, y1, in_sem, out_sem, p_sem, z_sem):
        sbufs = (s0, s1); ybufs = (y0, y1)
        zv = [None]; zs = [None]; fences = []; clock = [0]
        loads = [0, 0, 0, 0]
        pend = []
        def set_z(i):
            if i is None:
                zv[0] = None; zs[0] = None
            else:
                zs[0] = lax.shift_right_logical(i, 16)
                zv[0] = jnp.full((8, 128), zs[0], i32)
            fences.clear()
            loads[:] = [0, 0, 0, 0]
            return zs[0]

        def in_copies(hq, hkv, slot):
            return [pltpu.make_async_copy(src.at[hh], inb.at[slot, i, pl.ds(0, D)], in_sem.at[slot])
                    for i, src, hh in ((QI, q_hbm, hq), (KI, k_hbm, hkv), (VI, v_hbm, hkv))]

        def in_wait(slot):
            pltpu.make_async_copy(inb.at[slot, :, pl.ds(0, D)], inb.at[slot, :, pl.ds(0, D)], in_sem.at[slot]).wait()

        def out_copy(h, slot):
            return pltpu.make_async_copy(outb.at[slot], o_hbm.at[h], out_sem.at[slot])

        def tree(parts, op):
            parts = list(parts)
            while len(parts) > 1:
                nxt = [op(parts[i], parts[i + 1]) for i in range(0, len(parts) - 1, 2)]
                if len(parts) % 2: nxt.append(parts[-1])
                parts = nxt
            return parts[0]

        def tred(x, op):
            return tree([x[i * 8:(i + 1) * 8] for i in range(x.shape[0] // 8)], op)

        bits = lambda x: lax.bitcast_convert_type(x, i32)
        def zrow(align=8):
            return pl.ds(pl.multiple_of(zs[0] * align, align), 8)

        def add_fence(lag, tok):
            fences.append((clock[0] + lag, tok))

        def take_fences(all_=False):
            due = [t for (d, t) in fences if all_ or d <= clock[0]]
            fences[:] = [(d, t) for (d, t) in fences if not (all_ or d <= clock[0])]
            if not due: return None
            return lax.bitcast_convert_type(tree(due, jnp.bitwise_or) & zv[0], u32)

        def fenced(a, tok):
            if tok is not None:
                a = jnp.concatenate([a[0:8] | tok, a[8:]], axis=0)
            return pltpu.bitcast(a, bf16)

        def dsm(start, n, al):
            return pl.ds(start, n) if isinstance(start, int) else pl.ds(pl.multiple_of(start, al), n)

        def kprep_chunk(slot, ci, dst):
            c1 = dsm(2 * ci * r, r, 128); c2 = dsm(2 * ci * r + r, r, 128)
            k1 = inb[slot, KI, 0:D, c1].astype(f32); k2 = inb[slot, KI, 0:D, c2].astype(f32)
            a1t = jnp.concatenate([k1[0:64], k1[64:128] - k2[64:128]], axis=0)
            a2t = jnp.concatenate([k2[0:64], k2[128:192] - k1[128:192]], axis=0)
            a3t = jnp.concatenate([k2[64:128], k1[128:192]], axis=0)
            for i, x in enumerate((a1t, a2t, a3t)):
                dst[i, dsm(ci * (r // 2), r // 2, 8), :] = pltpu.bitcast(x.T.astype(bf16), u32)

        def vprep_col(slot, j, dst, rbs=range(hd // 16)):
            for rb in rbs:
                def blk(rr, cc):
                    return inb[slot, VI, pl.ds(rr * hd + rb * 16, 16), dsm(2 * j * r + cc * r, r, 128)]
                a11 = blk(0, 0); a22 = blk(1, 1)
                g11 = a11.astype(f32); g12 = blk(0, 1).astype(f32); g21 = blk(1, 0).astype(f32); g22 = a22.astype(f32)
                xs = [(g11 + g22).astype(bf16), (g21 + g22).astype(bf16), a11, a22, (g11 + g12).astype(bf16),
                      (g21 - g11).astype(bf16), (g12 - g22).astype(bf16)]
                for i in range(7):
                    dst[i, pl.ds(rb * 8, 8), dsm(j * r, r, 128)] = pltpu.bitcast(xs[i], u32)

        def stage(slot, kcs, vcs):
            def mk(kind, idx, rb):
                def f(anchor):
                    if gate and zs[0] is not None:
                        inb[slot, 0, pl.ds(pl.multiple_of(D + zs[0] * 16, 16), 16), 0:128] = anchor[0:16].astype(bf16)
                    if kind == 0: kprep_chunk(slot, idx, an_scr)
                    else: vprep_col(slot, idx, xn_scr, [rb])
                    if klag and zs[0] is not None:
                        if kind == 0: add_fence(klag, bits(an_scr[0, dsm(idx * (r // 2) + zs[0] * 8, 8, 8), :]))
                        elif rb == hd // 16 - 1: add_fence(klag, bits(xn_scr[0, zrow(), dsm(idx * r, r, 128)]))
                return f
            out = []
            for ci in kcs: out += [mk(0, ci, 0)] + [None] * kgap
            for j in vcs:
                for rb in range(hd // 16): out += [mk(1, j, rb)] + [None] * vgap
            return out

        def cols(u, off=0, n=w):
            if isinstance(u, int):
                return pl.ds(u * w + off, n)
            return pl.ds(pl.multiple_of(u * w + off, 128), n)

        def weights(slot, u, hh):
            qc = inb[slot, QI, 0:D, cols(u, hh * 128, 128)]
            return (qc[0:128], jnp.concatenate([qc[0:64], qc[128:192]], axis=0), qc[64:192])

        def trio(ws, s_ref, ci, hh):
            rows = pl.ds(ci * r // 2, r // 2)
            tok = take_fences() if zs[0] is not None else None
            m3 = jnp.dot(fenced(a_scr[2, rows, :], tok), ws[2], preferred_element_type=f32)
            m1 = jnp.dot(fenced(a_scr[0, rows, :], tok if f3 else None), ws[0], preferred_element_type=f32)
            m2 = jnp.dot(fenced(a_scr[1, rows, :], tok if f3 else None), ws[1], preferred_element_type=f32)
            for _ in range(3):
                loads[loads.index(min(loads))] += r
            s1_ = m1 + m3
            s2_ = m2 + m3
            if premul:
                s1_ = s1_ * c; s2_ = s2_ * c
            cs = pl.ds(hh * 128, 128)
            s_ref[pl.ds(2 * ci * r, r), cs] = s1_
            s_ref[pl.ds(2 * ci * r + r, r), cs] = s2_
            t = jnp.maximum(s1_, s2_).reshape(r // 8, 8, 128).max(axis=0)
            if zs[0] is not None and slag:
                add_fence(slag, bits(s_ref[zrow(), 0:128]) | bits(t))
            step_ = r // SPT
            return t, [bits(m3[i * step_:i * step_ + 8]) for i in range(SPT)]

        def fin_max(ts):
            m = jnp.max(tree(ts, jnp.maximum), axis=0, keepdims=True)
            if bal:
                cc = 2.0 if premul else 2.0 * c
                n2 = jnp.sum(tree([jnp.exp2((t - m) * cc) for t in ts], jnp.add), axis=0, keepdims=True)
                m = m + jnp.log2(n2) * (1.0 / cc)
            return jnp.broadcast_to(m, (8, 128))

        def sm_slab(par, k_, m8, l, anchor):
            s_ref = sbufs[par]; y_ref = ybufs[par]
            j, b = divmod(k_, SPC)
            mm = m8
            if anchor is not None:
                tk = anchor & zv[0]
                mm = lax.bitcast_convert_type(bits(m8) | jnp.concatenate([tk, tk], axis=1), f32)
            def ex(base):
                s = s_ref[pl.ds(base + b * slab, slab), :].reshape(slab // 8, 8, w)
                x = s - mm[None]
                if not premul: x = x * c
                return jnp.exp2(x).reshape(slab, w)
            p1 = ex(2 * j * r); p2 = ex(2 * j * r + r)
            t = tred(p1 + p2, jnp.add)
            b11 = p1[:, 0:128]; b12 = p1[:, 128:256]; b21 = p2[:, 0:128]; b22 = p2[:, 128:256]
            ys = [b11 - b22, b11, b22 - b12, b21 - b11, b22, b11 - b12, b21 - b22]
            for i in range(7):
                y_ref[i, pl.ds(j * r + b * slab, slab), :] = ys[i].astype(bf16)
            return t if l is None else l + t

        def y_fence(par, l):
            if zs[0] is not None and ylag:
                lb = bits(l)
                add_fence(ylag, bits(ybufs[par][0, zrow(16), :].astype(f32)) | lb[:, 0:128] | lb[:, 128:256])

        def queue_pv(pv, l_pv, vprep_slot, after=None):
            ms = [None] * 7
            def fin():
                m1, m2, m3, m4, m5, m6, m7 = ms
                rl = 1.0 / jnp.sum(l_pv, axis=0, keepdims=True)
                r1 = rl[:, 0:128]; r2 = rl[:, 128:256]
                c11 = (m1 + m4) + (m5 + m7); c12 = m5 - m3; c21 = m2 + m4; c22 = (m2 - m1) - (m3 + m6)
                outb[pv[0], 0:hd, cols(pv[1], 0, 128)] = (c11 * r1).astype(bf16)
                outb[pv[0], hd:D, cols(pv[1], 0, 128)] = (c21 * r1).astype(bf16)
                outb[pv[0], 0:hd, cols(pv[1], 128, 128)] = (c12 * r2).astype(bf16)
                outb[pv[0], hd:D, cols(pv[1], 128, 128)] = (c22 * r2).astype(bf16)
                if after is not None: after()
            def mk(i, j, lastt):
                def f(tok):
                    ks = pl.ds(j * r, r)
                    o = jnp.dot(fenced(x_scr[i, :, ks], tok), ybufs[pv[2]][i, ks, :], preferred_element_type=f32)
                    ms[i] = o if ms[i] is None else ms[i] + o
                    loads[loads.index(min(loads))] += hd
                    if vprep_slot: x_scr[i, :, ks] = xn_scr[i, :, ks]
                    if lastt: fin()
                    return o
                return f
            for n, i in enumerate(porder_):
                for j in range(NC):
                    pend.append(mk(i, j, n == 6 and j == NC - 1))

        def stepf(qk, sm, pv, st, kprep=None, vprep_slot=None, final=False, after=None, stg=None):
            m_sm, l_pv = st
            if pv is not None: queue_pv(pv, l_pv, vprep_slot, after)
            l = None; ms_new = []; ks = 0
            prev_anchors = []
            if qk is not None:
                for hh in range(2):
                    ws = weights(qk[0], qk[1], hh)
                    ts = []
                    for ci in range(NC):
                        clock[0] += 1
                        t, anc = trio(ws, sbufs[qk[2]], ci, hh)
                        ts.append(t)
                        if kprep and hh == 1:
                            rows = pl.ds(ci * r // 2, r // 2)
                            a_scr[:, rows, :] = an_scr[:, rows, :]
                        while pend and loads[3] < loads[0]:
                            pend.pop(0)(None)
                        if sm is not None:
                            for a in anc:
                                l = sm_slab(sm, ks, m_sm, l, a if (pace and zs[0] is not None) else None); ks += 1
                            y_fence(sm, l)
                    ms_new.append(fin_max(ts))
            n = 0
            while pend:
                if not final and qk is not None and len(pend) <= 3 and loads[0] == loads[1] == loads[2] and loads[3] >= loads[0]:
                    break
                if n % 4 == 0: clock[0] += 1
                n += 1
                tok = None
                if zs[0] is not None:
                    tok = take_fences(all_=(final and len(pend) == 1))
                o = pend.pop(0)(tok)
                if stg and not noprep and n >= ppos:
                    ff = stg.pop(0)
                    if ff is not None: ff(o)
                if sm is not None and ks < NC * SPC:
                    for e_ in range(etile + (1 if (etile == 1 and n % 4 == 0) else 0)):
                        if ks < NC * SPC:
                            l = sm_slab(sm, ks, m_sm, l, bits(o[e_ * 48:e_ * 48 + 8]) if zs[0] is not None else None); ks += 1
                    if n % 4 == 0: y_fence(sm, l)
            assert noprep or not any(stg or []), len(stg)
            while sm is not None and ks < NC * SPC:
                l = sm_slab(sm, ks, m_sm, l, None); ks += 1
            return ((jnp.concatenate(ms_new, axis=1) if qk is not None else None), l)

        kw = S // ksplit
        cks = [pltpu.make_async_copy(k_hbm.at[0, :, pl.ds(i * kw, kw)], inb.at[1, KI, pl.ds(0, D), pl.ds(i * kw, kw)], p_sem.at[5 + i])
               for i in range(ksplit)]
        def qcopy(a, b, sem):
            return pltpu.make_async_copy(q_hbm.at[0, :, pl.ds(a * w, (b - a) * w)], inb.at[0, QI, pl.ds(0, D), pl.ds(a * w, (b - a) * w)], p_sem.at[sem])
        cq0 = qcopy(0, 2, 0); cq1 = qcopy(2, 3, 1); cq2 = qcopy(3, 5, 0); cq3 = qcopy(5, NU, 1)
        cv = pltpu.make_async_copy(v_hbm.at[0], inb.at[1, VI, pl.ds(0, D)], p_sem.at[2])
        def hcopy(src, i, hf, sem):
            return pltpu.make_async_copy(src.at[1, :, pl.ds(hf * half, half)], inb.at[0, i, pl.ds(0, D), pl.ds(hf * half, half)], p_sem.at[sem])
        ck1 = hcopy(k_hbm, KI, 0, 3); cv1 = hcopy(v_hbm, VI, 0, 4); ck1b = hcopy(k_hbm, KI, 1, 2); cv1b = hcopy(v_hbm, VI, 1, 5)
        cks[0].start(); cq0.start()
        for cp in cks[1:]: cp.start()
        cv.start(); cq1.start()
        zz = pl.semaphore_read(z_sem) if zmode == 1 else None
        cks[0].wait(); cq0.wait()
        set_z(zz)
        wss = [weights(0, 0, hh) for hh in range(2)]
        tss = [[], []]
        for ci in range(NC):
            if ci > 0 and (ci * ksplit) % NC == 0:
                cks[ci * ksplit // NC].wait()
                set_z(zz)
            kprep_chunk(1, ci, a_scr)
            for hh in range(2):
                clock[0] += 1
                tss[hh].append(trio(wss[hh], sbufs[0], ci, hh)[0])
        st = (jnp.concatenate([fin_max(t) for t in tss], axis=1), None)
        st = stepf((0, 1, 1), 0, None, st)
        cv.wait(); cq1.wait()
        cq2.start(); ck1.start(); cv1.start(); cq3.start(); ck1b.start(); cv1b.start()
        set_z(zz)
        for j in range(NC): vprep_col(1, j, x_scr)
        st = stepf((0, 2, 0), 1, (0, 0, 0), st, final=True)
        cq2.wait(); ck1.wait(); cv1.wait()
        for cp in in_copies(1, 2, 1): cp.start()
        def pit(i, st):
            g = 2 * i + 1
            set_z(i)
            @pl.when(i == 1)
            def _():
                cq3.wait(); ck1b.wait(); cv1b.wait()
            st = stepf((0, g + 2, 1), 0, (0, g, 1), st, stg=stage(0, [4 * i, 4 * i + 1], [4 * i, 4 * i + 1]))
            st = stepf((0, g + 3, 0), 1, (0, g + 1, 0), st, final=True, stg=stage(0, [4 * i + 2, 4 * i + 3], [4 * i + 2, 4 * i + 3]))
            return st
        st = lax.fori_loop(0, 2, pit, st)

        def step(h, carry):
            st, _ = carry
            cur = h & 1; nx = 1 - cur
            z0 = set_z(h)
            in_wait(nx)
            @pl.when(h > 0)
            def _():
                out_copy(h - 1, nx).wait()
            st = stepf((cur, 7, 1), 0, (cur, 5, 1), st, kprep=True, stg=stage(nx, [0], []))
            for cp in in_copies(jnp.minimum(h + 2, H - 1), jnp.minimum(h + 3, H - 1), cur): cp.start()
            st = stepf((nx, 0, 0), 1, (cur, 6, 0), st, stg=stage(nx, [1, 2], []))
            st = stepf((nx, 1, 1), 0, (cur, 7, 1), st, vprep_slot=True,
                       after=lambda: out_copy(h, cur).start(), stg=stage(nx, [3, 4], []))
            vc = [[0, 1], [2, 3], [4], [5], [6, 7]]
            kc_ = [[], [], [5, 6], [7], []]
            for g in range(5):
                st = stepf((nx, g + 2, g % 2), (g + 1) % 2, (nx, g, g % 2), st, final=(g == 4), stg=stage(nx, kc_[g], vc[g]))
            return st, z0
        st, zc = lax.fori_loop(0, H - 1, step, (st, jnp.int32(0)))
        last = (H - 1) % 2

        set_z(zc)
        def ocopy(a, b, sem):
            return pltpu.make_async_copy(outb.at[last, :, pl.ds(a * w, (b - a) * w)], o_hbm.at[H - 1, :, pl.ds(a * w, (b - a) * w)], p_sem.at[sem])
        e0 = ocopy(0, 5, 0); e1 = ocopy(5, 7, 1); e2 = ocopy(7, 8, 2)
        e0.start()
        st = stepf((last, 7, 1), 0, (last, 5, 1), st, final=True)
        st = stepf(None, 1, (last, 6, 0), st, final=True)
        e1.start()
        stepf(None, None, (last, 7, 1), st, final=True)
        e2.start()
        in_wait(1 - last)
        out_copy(H - 2, 1 - last).wait()
        e0.wait(); e1.wait(); e2.wait()

    ot = pl.pallas_call(
        body,
        in_specs=[pl.BlockSpec(memory_space=pl.ANY)] * 3,
        out_specs=pl.BlockSpec(memory_space=pl.ANY),
        out_shape=jax.ShapeDtypeStruct((H, D, S), bf16),
        scratch_shapes=[
            pltpu.VMEM((2, 3, D + 16, S), bf16), pltpu.VMEM((2, D, S), bf16),
            pltpu.VMEM((3, half // 2, 128), u32), pltpu.VMEM((7, hd // 2, half), u32),
            pltpu.VMEM((3, half // 2, 128), u32), pltpu.VMEM((7, hd // 2, half), u32),
            pltpu.VMEM((S, w), f32), pltpu.VMEM((S, w), f32),
            pltpu.VMEM((7, half, 128), bf16), pltpu.VMEM((7, half, 128), bf16),
            pltpu.SemaphoreType.DMA((2,)), pltpu.SemaphoreType.DMA((2,)), pltpu.SemaphoreType.DMA((5 + ksplit,)), pltpu.SemaphoreType.REGULAR,
        ],
        compiler_params=pltpu.CompilerParams(
            vmem_limit_bytes=100 * 1024 * 1024, disable_bounds_checks=bool(nobc)),
    )(qt, kt, vt)
    return jnp.swapaxes(ot.reshape(B, H, D, S), 2, 3)
```

```python
import math

import jax
import jax.numpy as jnp
from jax import lax
import jax.experimental.pallas as pl
import jax.experimental.pallas.tpu as pltpu

f32 = jnp.float32
bf16 = jnp.bfloat16
i32 = jnp.int32
u32 = jnp.uint32

W = 256
R = 128
SLAB = 16
YLAG, SLAG, KLAG = 5, 4, 9
PORDER = (1, 3, 0, 2, 4, 5, 6)


def _tree(parts, op):
    parts = list(parts)
    while len(parts) > 1:
        nxt = [op(parts[i], parts[i + 1]) for i in range(0, len(parts) - 1, 2)]
        if len(parts) % 2:
            nxt.append(parts[-1])
        parts = nxt
    return parts[0]


def _bits(x):
    return lax.bitcast_convert_type(x, i32)


def _ds(start, n, align):
    if isinstance(start, int):
        return pl.ds(start, n)
    return pl.ds(pl.multiple_of(start, align), n)


@jax.jit
def pallas_standalone__mha_softmax__prompt_kernel(q: jax.Array, k: jax.Array, v: jax.Array):
    B, NH, S, D = q.shape
    H = B * NH
    assert D == 192 and S == 2048 and H >= 3 and k.shape == q.shape and v.shape == q.shape
    qt = jnp.swapaxes(q, 2, 3).reshape(H, D, S)
    kt = jnp.swapaxes(k, 2, 3).reshape(H, D, S)
    vt = jnp.swapaxes(v, 2, 3).reshape(H, D, S)
    c = (D ** -0.5) * math.log2(math.e)
    hd = D // 2
    half = S // 2
    NU = S // W
    NC = S // (2 * R)
    SPC = R // SLAB
    SPT = SPC // 2
    NRB = hd // 16
    KI, VI = 0, 1

    def body(q_hbm, k_hbm, v_hbm, o_hbm, qb, kvb, outb, a_scr, x_scr, an_scr, xn_scr,
             s0, s1, y0, y1, q_sem, kv_sem, out_sem, p_sem):
        sbufs = (s0, s1)
        ybufs = (y0, y1)
        zero = {}
        fences = []
        clock = [0]
        loads = [0, 0, 0, 0]
        pend = []

        def new_block(i):
            zero["s"] = lax.shift_right_logical(i, 16)
            zero["v"] = jnp.full((8, R), zero["s"], i32)
            fences.clear()
            loads[:] = [0, 0, 0, 0]
            return zero["s"]

        def zrows(base=0, n=8, align=8):
            return pl.ds(pl.multiple_of(base + zero["s"] * align, align), n)

        def add_fence(lag, tok):
            fences.append((clock[0] + lag, tok))

        def take_fences(flush=False):
            due = [t for (d, t) in fences if flush or d <= clock[0]]
            fences[:] = [(d, t) for (d, t) in fences if not (flush or d <= clock[0])]
            if not due:
                return None
            return lax.bitcast_convert_type(_tree(due, jnp.bitwise_or) & zero["v"], u32)

        def lhs(a, tok):
            if tok is not None:
                a = jnp.concatenate([a[0:8] | tok, a[8:]], axis=0)
            return pltpu.bitcast(a, bf16)

        def in_copies(hq, hkv, slot):
            return [pltpu.make_async_copy(q_hbm.at[hq], qb.at[slot], q_sem.at[slot])] + [
                pltpu.make_async_copy(src.at[hkv], kvb.at[slot, i, pl.ds(0, D)], kv_sem.at[slot])
                for i, src in ((KI, k_hbm), (VI, v_hbm))]

        def in_wait(slot):
            pltpu.make_async_copy(qb.at[slot], qb.at[slot], q_sem.at[slot]).wait()
            both = kvb.at[slot, :, pl.ds(0, D)]
            pltpu.make_async_copy(both, both, kv_sem.at[slot]).wait()

        def out_copy(h, slot):
            return pltpu.make_async_copy(outb.at[slot], o_hbm.at[h], out_sem.at[slot])

        def kprep(slot, ci, dst):
            k1 = kvb[slot, KI, 0:D, _ds(2 * ci * R, R, R)].astype(f32)
            k2 = kvb[slot, KI, 0:D, _ds(2 * ci * R + R, R, R)].astype(f32)
            a1t = jnp.concatenate([k1[0:64], k1[64:128] - k2[64:128]], axis=0)
            a2t = jnp.concatenate([k2[0:64], k2[128:192] - k1[128:192]], axis=0)
            a3t = jnp.concatenate([k2[64:128], k1[128:192]], axis=0)
            for i, x in enumerate((a1t, a2t, a3t)):
                dst[i, _ds(ci * (R // 2), R // 2, 8), :] = pltpu.bitcast(x.T.astype(bf16), u32)

        def vprep(slot, j, rb, dst):
            def blk(rr, cc):
                return kvb[slot, VI, pl.ds(rr * hd + rb * 16, 16), _ds(2 * j * R + cc * R, R, R)]
            a11 = blk(0, 0)
            a22 = blk(1, 1)
            g11 = a11.astype(f32)
            g12 = blk(0, 1).astype(f32)
            g21 = blk(1, 0).astype(f32)
            g22 = a22.astype(f32)
            xs = [(g11 + g22).astype(bf16), (g21 + g22).astype(bf16), a11, a22,
                  (g11 + g12).astype(bf16), (g21 - g11).astype(bf16), (g12 - g22).astype(bf16)]
            for i in range(7):
                dst[i, pl.ds(rb * 8, 8), _ds(j * R, R, R)] = pltpu.bitcast(xs[i], u32)

        def stage(slot, kcs, vps, kgap, vgap, interleave=False):
            def mk(kind, idx, rb=0, fence=True):
                def f(anchor):
                    kvb[slot, 0, zrows(D, 16, 16), 0:R] = anchor[0:16].astype(bf16)
                    if kind == 0:
                        kprep(slot, idx, an_scr)
                        add_fence(KLAG, _bits(an_scr[0, zrows(idx * (R // 2)), :]))
                    else:
                        vprep(slot, idx, rb, xn_scr)
                        if fence:
                            add_fence(KLAG, _bits(xn_scr[0, zrows(rb * 8), _ds(idx * R, R, R)]))
                return f
            out = []
            if not interleave:
                for ci in kcs:
                    out += [mk(0, ci)] + [None] * kgap
            for n, (j, rb) in enumerate(vps):
                out += [mk(1, j, rb, n % 4 == 3 or n == len(vps) - 1)] + [None] * vgap
            if interleave:
                for n, ci in enumerate(kcs):
                    out[1 + n * kgap] = mk(0, ci)
            return out

        def weights(slot, u, hh):
            qc = qb[slot, :, _ds(u * W + hh * R, R, R)]
            return (qc[0:128], jnp.concatenate([qc[0:64], qc[128:192]], axis=0), qc[64:192])

        def trio(ws, s_ref, ci, hh):
            rows = pl.ds(ci * R // 2, R // 2)
            tok = take_fences()
            m3 = jnp.dot(lhs(a_scr[2, rows, :], tok), ws[2], preferred_element_type=f32)
            m1 = jnp.dot(lhs(a_scr[0, rows, :], tok), ws[0], preferred_element_type=f32)
            m2 = jnp.dot(lhs(a_scr[1, rows, :], tok), ws[1], preferred_element_type=f32)
            for _ in range(3):
                loads[loads.index(min(loads))] += R
            sa = (m1 + m3) * c
            sb = (m2 + m3) * c
            cs = pl.ds(hh * R, R)
            s_ref[2 * ci, :, cs] = sa
            s_ref[2 * ci + 1, :, cs] = sb
            t = jnp.maximum(sa, sb).reshape(R // 8, 8, R).max(axis=0)
            add_fence(SLAG, _bits(s_ref[0, zrows(), 0:R]) | _bits(t))
            gap = R // SPT
            return t, [_bits(m3[i * gap:i * gap + 8]) for i in range(SPT)]

        def row_shift(ts):
            m = jnp.max(_tree(ts, jnp.maximum), axis=0, keepdims=True)
            n2 = jnp.sum(_tree([jnp.exp2((t - m) * 2.0) for t in ts], jnp.add), axis=0, keepdims=True)
            return jnp.broadcast_to(m + jnp.log2(n2) * 0.5, (8, R))

        def sm_slab(par, idx, m8, l, anchor):
            j, b = divmod(idx, SPC)
            tk = anchor & zero["v"]
            mm = lax.bitcast_convert_type(_bits(m8) | jnp.concatenate([tk, tk], axis=1), f32)
            s = sbufs[par][pl.ds(2 * j, 2), pl.ds(b * SLAB, SLAB), :]
            p = jnp.exp2(s.reshape(2 * SLAB // 8, 8, W) - mm[None]).reshape(2 * SLAB, W)
            ps = p[0:SLAB] + p[SLAB:2 * SLAB]
            t = ps[0:8] + ps[8:16]
            b11 = p[0:SLAB, 0:R]
            b12 = p[0:SLAB, R:W]
            b21 = p[SLAB:2 * SLAB, 0:R]
            b22 = p[SLAB:2 * SLAB, R:W]
            ys = jnp.concatenate([b11 - b22, b11, b22 - b12, b21 - b11, b22, b11 - b12, b21 - b22], axis=0)
            ybufs[par][:, pl.ds(j * R + b * SLAB, SLAB), :] = ys.astype(bf16).reshape(7, SLAB, R)
            return t if l is None else l + t

        def y_fence(par, l):
            lb = _bits(l)
            add_fence(YLAG, _bits(ybufs[par][0, zrows(0, 8, 16), :].astype(f32)) | lb[:, 0:R] | lb[:, R:W])

        def queue_pv(pv, l_pv, swap_x, after):
            slot, u, par = pv
            ms = [None] * 7

            def finish():
                m1, m2, m3, m4, m5, m6, m7 = ms
                rl = 1.0 / jnp.sum(l_pv, axis=0, keepdims=True)
                r1 = rl[:, 0:R]
                r2 = rl[:, R:W]
                c11 = (m1 + m4) + (m5 + m7)
                c12 = m5 - m3
                c21 = m2 + m4
                c22 = (m2 - m1) - (m3 + m6)
                outb[slot, 0:hd, _ds(u * W, R, R)] = (c11 * r1).astype(bf16)
                outb[slot, hd:D, _ds(u * W, R, R)] = (c21 * r1).astype(bf16)
                outb[slot, 0:hd, _ds(u * W + R, R, R)] = (c12 * r2).astype(bf16)
                outb[slot, hd:D, _ds(u * W + R, R, R)] = (c22 * r2).astype(bf16)
                if after is not None:
                    after()

            def mk(i, j, last):
                def f(tok):
                    ks = pl.ds(j * R, R)
                    o = jnp.dot(lhs(x_scr[i, :, ks], tok), ybufs[par][i, ks, :], preferred_element_type=f32)
                    ms[i] = o if ms[i] is None else ms[i] + o
                    loads[loads.index(min(loads))] += hd
                    if swap_x:
                        x_scr[i, :, ks] = xn_scr[i, :, ks]
                    if last:
                        finish()
                    return o
                return f

            for n, i in enumerate(PORDER):
                for j in range(NC):
                    pend.append(mk(i, j, n == 6 and j == NC - 1))

        def step(qk, sm, pv, st, swap_a=False, swap_x=False, final=False, after=None, stg=None):
            m_sm, l_pv = st
            if pv is not None:
                queue_pv(pv, l_pv, swap_x, after)
            l = None
            shifts = []
            ns = 0
            if qk is not None:
                for hh in range(2):
                    ws = weights(qk[0], qk[1], hh)
                    ts = []
                    for ci in range(NC):
                        clock[0] += 1
                        t, anchors = trio(ws, sbufs[qk[2]], ci, hh)
                        ts.append(t)
                        if swap_a and hh == 1:
                            rows = pl.ds(ci * R // 2, R // 2)
                            a_scr[:, rows, :] = an_scr[:, rows, :]
                        while pend and loads[3] < loads[0]:
                            pend.pop(0)(None)
                        for a in anchors:
                            l = sm_slab(sm, ns, m_sm, l, a)
                            ns += 1
                        y_fence(sm, l)
                    shifts.append(row_shift(ts))
            n = 0
            while pend:
                if (not final and len(pend) <= 3
                        and loads[0] == loads[1] == loads[2] and loads[3] >= loads[0]):
                    break
                if n % 4 == 0:
                    clock[0] += 1
                n += 1
                o = pend.pop(0)(take_fences(flush=(final and len(pend) == 1)))
                if stg:
                    piece = stg.pop(0)
                    if piece is not None:
                        piece(o)
                if sm is not None and ns < NC * SPC:
                    for e in range(2 if n % 4 == 0 else 1):
                        if ns < NC * SPC:
                            l = sm_slab(sm, ns, m_sm, l, _bits(o[e * 48:e * 48 + 8]))
                            ns += 1
                    if n % 4 == 0:
                        y_fence(sm, l)
            assert not any(stg or []) and (sm is None or ns == NC * SPC)
            return (jnp.concatenate(shifts, axis=1) if qk is not None else None), l

        def qcopy(a, b, sem):
            cs = pl.ds(a * W, (b - a) * W)
            return pltpu.make_async_copy(q_hbm.at[0, :, cs], qb.at[0, :, cs], p_sem.at[sem])

        def hcopy(src, h, slot, i, hf, sem):
            cs = pl.ds(hf * half, half)
            return pltpu.make_async_copy(src.at[h, :, cs], kvb.at[slot, i, pl.ds(0, D), cs], p_sem.at[sem])

        ck0a = hcopy(k_hbm, 0, 1, KI, 0, 5)
        ck0b = hcopy(k_hbm, 0, 1, KI, 1, 6)
        cq0, cq1, cq2, cq3 = qcopy(0, 2, 0), qcopy(2, 3, 1), qcopy(3, 5, 0), qcopy(5, NU, 1)
        cv0 = pltpu.make_async_copy(v_hbm.at[0], kvb.at[1, VI, pl.ds(0, D)], p_sem.at[2])
        ck1a, cv1a = hcopy(k_hbm, 1, 0, KI, 0, 3), hcopy(v_hbm, 1, 0, VI, 0, 4)
        ck1b, cv1b = hcopy(k_hbm, 1, 0, KI, 1, 2), hcopy(v_hbm, 1, 0, VI, 1, 5)
        for cp in (ck0a, cq0, ck0b, cv0, cq1):
            cp.start()
        small = lax.fori_loop(0, 3, lambda i, acc: acc + i, jnp.int32(0))
        ck0a.wait()
        cq0.wait()
        new_block(small)
        wss = [weights(0, 0, hh) for hh in range(2)]
        tss = [[], []]
        for ci in range(NC):
            if ci == NC // 2:
                ck0b.wait()
                new_block(small)
            kprep(1, ci, a_scr)
            for hh in range(2):
                clock[0] += 1
                tss[hh].append(trio(wss[hh], sbufs[0], ci, hh)[0])
        st = (jnp.concatenate([row_shift(t) for t in tss], axis=1), None)
        st = step((0, 1, 1), 0, None, st)
        cv0.wait()
        cq1.wait()
        for cp in (cq2, ck1a, cv1a, cq3, ck1b, cv1b):
            cp.start()
        new_block(small)
        for j in range(NC):
            for rb in range(NRB):
                vprep(1, j, rb, x_scr)
        st = step((0, 2, 0), 1, (0, 0, 0), st, final=True)
        cq2.wait()
        ck1a.wait()
        cv1a.wait()
        for cp in in_copies(1, 2, 1):
            cp.start()

        def warm(i, st):
            g = 2 * i + 1
            new_block(i)

            @pl.when(i == 1)
            def _():
                cq3.wait()
                ck1b.wait()
                cv1b.wait()

            def stg(e):
                cs = [4 * i + e, 4 * i + e + 1]
                return stage(0, cs, [(j, rb) for j in cs for rb in range(NRB)], 8, 1, True)

            st = step((0, g + 2, 1), 0, (0, g, 1), st, stg=stg(0))
            return step((0, g + 3, 0), 1, (0, g + 1, 0), st, final=True, stg=stg(2))

        st = lax.fori_loop(0, 2, warm, st)

        def head(h, carry):
            st, _ = carry
            cur = h & 1
            nx = 1 - cur
            z = new_block(h)
            in_wait(nx)

            @pl.when(h > 0)
            def _():
                out_copy(h - 1, nx).wait()

            st = step((cur, 7, 1), 0, (cur, 5, 1), st, swap_a=True, stg=stage(nx, [0, 1, 2], [], 9, 2))
            for cp in in_copies(jnp.minimum(h + 2, H - 1), jnp.minimum(h + 3, H - 1), cur):
                cp.start()
            st = step((nx, 0, 0), 1, (cur, 6, 0), st, stg=stage(nx, [3, 4, 5], [], 9, 2))
            st = step((nx, 1, 1), 0, (cur, 7, 1), st, swap_x=True,
                      after=lambda: out_copy(h, cur).start(), stg=stage(nx, [6, 7], [], 9, 2))
            vall = [(j, rb) for j in range(NC) for rb in range(NRB)]
            for g in range(5):
                st = step((nx, g + 2, g % 2), (g + 1) % 2, (nx, g, g % 2), st, final=(g == 4),
                          stg=stage(nx, [], vall[10 * g:10 * g + 10], 9, 2))
            return st, z

        st, z = lax.fori_loop(0, H - 1, head, (st, jnp.int32(0)))

        last = (H - 1) % 2
        new_block(z)

        def ocopy(a, b, sem):
            cs = pl.ds(a * W, (b - a) * W)
            return pltpu.make_async_copy(outb.at[last, :, cs], o_hbm.at[H - 1, :, cs], p_sem.at[sem])

        e0, e1, e2 = ocopy(0, 5, 0), ocopy(5, 7, 1), ocopy(7, 8, 2)
        e0.start()
        st = step((last, 7, 1), 0, (last, 5, 1), st, final=True)
        st = step(None, 1, (last, 6, 0), st, final=True)
        e1.start()
        step(None, None, (last, 7, 1), st, final=True)
        e2.start()
        in_wait(1 - last)
        out_copy(H - 2, 1 - last).wait()
        e0.wait()
        e1.wait()
        e2.wait()

    ot = pl.pallas_call(
        body,
        in_specs=[pl.BlockSpec(memory_space=pl.ANY)] * 3,
        out_specs=pl.BlockSpec(memory_space=pl.ANY),
        out_shape=jax.ShapeDtypeStruct((H, D, S), bf16),
        scratch_shapes=[
            pltpu.VMEM((2, D, S), bf16),
            pltpu.VMEM((2, 2, D + 16, S), bf16),
            pltpu.VMEM((2, D, S), bf16),
            pltpu.VMEM((3, half // 2, R), u32),
            pltpu.VMEM((7, hd // 2, half), u32),
            pltpu.VMEM((3, half // 2, R), u32),
            pltpu.VMEM((7, hd // 2, half), u32),
            pltpu.VMEM((2 * NC, R, W), f32),
            pltpu.VMEM((2 * NC, R, W), f32),
            pltpu.VMEM((7, half, R), bf16),
            pltpu.VMEM((7, half, R), bf16),
            pltpu.SemaphoreType.DMA((2,)),
            pltpu.SemaphoreType.DMA((2,)),
            pltpu.SemaphoreType.DMA((2,)),
            pltpu.SemaphoreType.DMA((7,)),
        ],
        compiler_params=pltpu.CompilerParams(vmem_limit_bytes=64 * 1024 * 1024),
    )(qt, kt, vt)
    return jnp.swapaxes(ot.reshape(B, NH, D, S), 2, 3)
```

```python
import itertools
import math

import jax
import jax.numpy as jnp
from jax import lax
import jax.experimental.pallas as pl
import jax.experimental.pallas.tpu as pltpu

f32 = jnp.float32
bf16 = jnp.bfloat16
i32 = jnp.int32
u32 = jnp.uint32

W = 512
R = 128
SLAB = 16
NP = 26
T = (-1.375, -0.328125, 0.328125, 1.375)
PAIRS = tuple(itertools.combinations(range(4), 2))
BS = {(0, 1): 1.0, (0, 2): 1.0, (0, 3): -1.0, (1, 2): -1.0, (1, 3): 1.0, (2, 3): 1.0}
YLAG, SLAG, KLAG, CLAG, ELAG, NST = 6, 5, 9, 4, 3, 52


def _tree(parts, op):
    parts = list(parts)
    while len(parts) > 1:
        nxt = [op(parts[i], parts[i + 1]) for i in range(0, len(parts) - 1, 2)]
        if len(parts) % 2:
            nxt.append(parts[-1])
        parts = nxt
    return parts[0]


def _bits(x):
    return lax.bitcast_convert_type(x, i32)


def _spread(pieces, slots):
    for n, piece in enumerate(pieces):
        slots[n * len(slots) // len(pieces)].append(piece)


@jax.jit
def pallas_standalone__mha_softmax__prompt_kernel(q: jax.Array, k: jax.Array, v: jax.Array):
    B, NH, S, D = q.shape
    H = B * NH
    assert D == 192 and S == 2048 and H >= 3 and k.shape == q.shape and v.shape == q.shape
    qt = jnp.swapaxes(q, 2, 3).reshape(H, D, S)
    kt = jnp.swapaxes(k, 2, 3).reshape(H, D, S)
    vt = jnp.swapaxes(v, 2, 3).reshape(H, D, S)
    c = (D ** -0.5) * math.log2(math.e)
    hd = D // 2
    half = S // 2
    NC = S // (2 * R)
    NG = S // (4 * R)
    NQ = W // R
    SPG = R // SLAB
    NRB = hd // 16

    def body(q_hbm, k_hbm, v_hbm, o_hbm, qb, kb, vb, outb, a_scr, x_scr, an_scr, xn_scr,
             s0, s1, y0, y1, m0, m1, q_sem, k_sem, v_sem, out_sem, p_sem):
        sbufs = (s0, s1)
        ybufs = (y0, y1)
        mbufs = (m0, m1)
        zero = {}
        fences = []
        clock = [0]
        loads = [0, 0, 0, 0]
        pend = []

        def new_block(i):
            zero["s"] = lax.shift_right_logical(i, 16)
            zero["v"] = jnp.full((8, R), zero["s"], i32)
            fences.clear()
            loads[:] = [0, 0, 0, 0]

        def zrows(base=0, n=8, align=8):
            return pl.ds(pl.multiple_of(base + zero["s"] * align, align), n)

        def add_fence(lag, tok):
            fences.append((clock[0] + lag, tok, clock[0]))

        def take_fences(flush=False):
            def ok(x):
                return x[0] <= clock[0] or (flush and x[2] + 3 <= clock[0])
            due = [x[1] for x in fences if ok(x)]
            fences[:] = [x for x in fences if not ok(x)]
            if not due:
                return None
            return lax.bitcast_convert_type(_tree(due, jnp.bitwise_or) & zero["v"], u32)

        def lhs(a, tok):
            if tok is not None:
                a = jnp.concatenate([a[0:8] | tok, a[8:]], axis=0)
            return pltpu.bitcast(a, bf16)

        def q_copy(h, slot):
            return pltpu.make_async_copy(q_hbm.at[h], qb.at[slot], q_sem.at[slot])

        def k_copy(h, slot):
            return pltpu.make_async_copy(k_hbm.at[h], kb.at[slot, pl.ds(0, D)], k_sem.at[slot])

        def v_copy(h, slot):
            return pltpu.make_async_copy(v_hbm.at[h], vb.at[slot, pl.ds(0, D)], v_sem.at[slot])

        def out_copy(h, slot):
            return pltpu.make_async_copy(outb.at[slot], o_hbm.at[h], out_sem.at[slot])

        def kprep(slot, ci, dst):
            k1 = kb[slot, 0:D, pl.ds(2 * ci * R, R)].astype(f32)
            k2 = kb[slot, 0:D, pl.ds(2 * ci * R + R, R)].astype(f32)
            a1t = jnp.concatenate([k1[0:64], k1[64:128] - k2[64:128]], axis=0)
            a2t = jnp.concatenate([k2[0:64], k2[128:192] - k1[128:192]], axis=0)
            a3t = jnp.concatenate([k2[64:128], k1[128:192]], axis=0)
            for i, x in enumerate((a1t, a2t, a3t)):
                dst[i, pl.ds(ci * (R // 2), R // 2), :] = pltpu.bitcast(x.T.astype(bf16), u32)

        def vprep(slot, g, rb, e, dst):
            def blk(rr, kk):
                return vb[slot, pl.ds(rr * hd + rb * 16, 16), pl.ds((4 * g + kk) * R, R)]

            def put(r, x):
                dst[r, g, pl.ds(rb * 8, 8), :] = pltpu.bitcast(x.astype(bf16), u32)

            if e == 6:
                for kk in range(4):
                    lo = blk(1, kk)
                    put(18 + 2 * kk, blk(0, kk).astype(f32) + T[kk] * lo.astype(f32))
                    put(19 + 2 * kk, lo)
                return
            kk, qq = PAIRS[e]
            b = BS[(kk, qq)]
            it = 1.0 / (T[qq] - T[kk])
            u1k = blk(0, kk).astype(f32)
            u2k = blk(1, kk).astype(f32)
            u1q = blk(0, qq).astype(f32)
            u2q = blk(1, qq).astype(f32)
            top = ((u1k + u1q) if b > 0 else (u1k - u1q)) * it
            xa = top + u2k * (T[qq] * it) + u2q * (b * T[qq] * it)
            put(3 * e, xa)
            xc = xa - u2k
            put(3 * e + 2, xc)
            put(3 * e + 1, (xc - u2q) if b > 0 else (xc + u2q))

        def k_piece(slot, ci):
            def f(anchor):
                kb[slot, zrows(D, 16, 16), 0:R] = anchor[0:16].astype(bf16)
                kprep(slot, ci, an_scr)
                add_fence(KLAG, _bits(an_scr[0, zrows(ci * (R // 2)), :]))
            return f

        def v_pieces(slot, vps, dst):
            def mk(g, rb, e, fence):
                def f(anchor):
                    vb[slot, zrows(D, 16, 16), 0:R] = anchor[0:16].astype(bf16)
                    vprep(slot, g, rb, e, dst)
                    if fence:
                        add_fence(KLAG, _bits(dst[3 * e, g, zrows(rb * 8), :]))
                return f
            return [mk(g, rb, e, n % 4 == 3 or n == len(vps) - 1) for n, (g, rb, e) in enumerate(vps)]

        def stage(kslot, kcs, vslot, vps, kgap=12):
            out = [[] for _ in range(NST)]
            for n, ci in enumerate(kcs):
                out[n * kgap].append(k_piece(kslot, ci))
            _spread(v_pieces(vslot, vps, xn_scr), out)
            return out

        def weights(slot, u, hh):
            qc = qb[slot, :, pl.ds(u * W + hh * R, R)]
            return (qc[0:128], jnp.concatenate([qc[0:64], qc[128:192]], axis=0), qc[64:192])

        def trio(ws, s_ref, ci, hh):
            rows = pl.ds(ci * R // 2, R // 2)
            tok = take_fences()
            m3 = jnp.dot(lhs(a_scr[2, rows, :], tok), ws[2], preferred_element_type=f32)
            m1 = jnp.dot(lhs(a_scr[0, rows, :], tok), ws[0], preferred_element_type=f32)
            m2 = jnp.dot(lhs(a_scr[1, rows, :], tok), ws[1], preferred_element_type=f32)
            for _ in range(3):
                loads[loads.index(min(loads))] += R
            sa = (m1 + m3) * c
            sb = (m2 + m3) * c
            s_ref[hh, 2 * ci] = sa
            s_ref[hh, 2 * ci + 1] = sb
            t = jnp.maximum(sa, sb).reshape(R // 8, 8, R).max(axis=0)
            add_fence(SLAG, _bits(s_ref[0, 0, zrows(), :]) | _bits(t))
            return t, m3

        def row_shift(ts):
            m = jnp.max(_tree(ts, jnp.maximum), axis=0, keepdims=True)
            n2 = jnp.sum(_tree([jnp.exp2((t - m) * 2.0) for t in ts], jnp.add), axis=0, keepdims=True)
            return jnp.broadcast_to(m + jnp.log2(n2) * 0.5, (8, R))

        def sm_slab(par, idx, m8, l, anchors):
            g, b = divmod(idx, SPG)
            rows = pl.ds(b * SLAB, SLAB)
            yrows = pl.ds(g * R + b * SLAB, SLAB)

            def mk_exp(anchor, qs):
                tk = _bits(anchor) & zero["v"]
                mm = {qq: lax.bitcast_convert_type(_bits(m8[qq]) | tk, f32) for qq in qs}

                def ex(kk, qq):
                    s = sbufs[par][qq, 4 * g + kk, rows, :]
                    return jnp.exp2(s.reshape(2, 8, R) - mm[qq][None]).reshape(SLAB, R)
                return ex

            def put(r, x):
                ybufs[par][r, yrows, :] = x.astype(bf16)

            def diff(kk, qq, pkq, pqk):
                put(3 * PAIRS.index((kk, qq)) + 2, pkq - pqk)

            def single(kk, qq, p):
                if kk < qq:
                    put(3 * PAIRS.index((kk, qq)), p)
                else:
                    put(3 * PAIRS.index((qq, kk)) + 1, p)

            uc = {}
            ur = {}
            for n, (i, j) in enumerate(((0, 3), (1, 2))):
                ex = mk_exp(anchors[n], (i, j))
                pii, pjj, pij, pji = ex(i, i), ex(j, j), ex(i, j), ex(j, i)
                single(i, j, pij)
                single(j, i, pji)
                diff(i, j, pij, pji)
                uc[i] = pii + pji
                uc[j] = pjj + pij
                ur[i] = pii + pij
                ur[j] = pjj + pji
            keep = {}
            l = list(l)
            for n, (rs, cs) in enumerate((((0, 3), (1, 2)), ((1, 2), (0, 3)))):
                ex = mk_exp(anchors[2 + n], cs)
                p = {(kk, qq): ex(kk, qq) for kk in rs for qq in cs}
                for (kk, qq), x in p.items():
                    single(kk, qq, x)
                for kk in rs:
                    put(19 + 2 * kk, ur[kk] - (p[(kk, cs[0])] + p[(kk, cs[1])]))
                for qq in cs:
                    vc = p[(rs[0], qq)] + p[(rs[1], qq)]
                    put(18 + 2 * qq, uc[qq] - vc)
                    tot = uc[qq] + vc
                    tot = tot[0:8] + tot[8:16]
                    l[qq] = tot if l[qq] is None else l[qq] + tot
                if n == 0:
                    keep = p
                else:
                    for (kk, qq), x in p.items():
                        if kk < qq:
                            diff(kk, qq, x, keep[(qq, kk)])
                        else:
                            diff(qq, kk, keep[(qq, kk)], x)
            return l

        def y_fence(par, l, lag):
            tok = _bits(ybufs[par][0, zrows(0, 8, 16), :].astype(f32))
            add_fence(lag, _tree([tok] + [_bits(x) for x in l], jnp.bitwise_or))

        def queue_pv(par, swap_x):
            ms = {}

            def mk(i, j):
                def f(tok, even=False):
                    yy = pltpu.bitcast(ybufs[par].bitcast(u32)[i, pl.ds(j * R // 2, R // 2), :], bf16)
                    xx = lhs(x_scr[i, j], tok)
                    if even:
                        assert loads[0] == loads[1] == loads[2] == loads[3] - hd // 3
                        o = jnp.concatenate(
                            [jnp.dot(xx[a:a + hd // 3], yy, preferred_element_type=f32)
                             for a in range(0, hd, hd // 3)], axis=0)
                    else:
                        o = jnp.dot(xx, yy, preferred_element_type=f32)
                    ms[i] = o if j == 0 else ms[i] + o
                    loads[loads.index(min(loads))] += hd
                    if swap_x and j % 2 == 1:
                        xn_scr[NP, 0, zrows(), :] = lax.bitcast_convert_type(o[0:8], u32)
                        for jj in (j - 1, j):
                            x_scr[i, jj] = xn_scr[i, jj]
                    if j == NG - 1:
                        mbufs[par][i] = ms[i]
                        add_fence(CLAG, _bits(mbufs[par][i, zrows(), :]))
                    return o
                return f

            for i in range(NP):
                for j in range(NG):
                    pend.append(mk(i, j))

        def fin_pieces(fin, l_fin):
            slot, u, par = fin
            m_ref = mbufs[par]
            rls = {}

            def mk(qq, rb):
                def f(anchor):
                    if anchor is not None:
                        m_ref[NP, zrows(), :] = anchor[0:8]
                    if qq not in rls:
                        rls[qq] = 1.0 / jnp.sum(l_fin[qq], axis=0, keepdims=True)

                    def prod(r):
                        return m_ref[r, pl.ds(rb * 16, 16), :]

                    gq = prod(19 + 2 * qq)
                    oth = []
                    for e, (i, j) in enumerate(PAIRS):
                        b = BS[(i, j)]
                        if qq == j:
                            oth.append((i, prod(3 * e), 1.0))
                            gq = gq - (prod(3 * e + 1) + prod(3 * e + 2))
                        elif qq == i:
                            d = prod(3 * e) - prod(3 * e + 2)
                            gq = (gq + d) if b > 0 else (gq - d)
                            oth.append((j, prod(3 * e + 1), -b))
                    c1 = prod(18 + 2 * qq) - gq * T[qq]
                    c2 = gq
                    for kk, gv, sg in oth:
                        c1 = c1 - gv * (T[kk] * sg)
                        c2 = (c2 + gv) if sg > 0 else (c2 - gv)
                    cols = pl.ds(u * W + qq * R, R)
                    outb[slot, pl.ds(rb * 16, 16), cols] = (c1 * rls[qq]).astype(bf16)
                    outb[slot, pl.ds(hd + rb * 16, 16), cols] = (c2 * rls[qq]).astype(bf16)
                    if anchor is not None and rb % 3 == 2:
                        add_fence(KLAG, _bits(outb[slot, zrows(rb * 16, 8, 16), cols].astype(f32)))
                return f
            return [mk(qq, rb) for qq in range(NQ) for rb in range(NRB)]

        def step(qk, sm, pv, fin, st, swap_a=False, swap_x=False, final=0, stg=None, qx=(), mid=None):
            m_sm, l_pv, l_fin = st
            if pv is not None:
                queue_pv(pv, swap_x)
            stg = stg or [[] for _ in range(NST)]
            qs = [[] for _ in range(NQ * NC)]
            _spread(list(qx), qs[:NQ * NC - 2])
            if fin is not None:
                fp = fin_pieces(fin, l_fin)
                if pv is None:
                    for piece in fp:
                        piece(None)
                elif qk is not None:
                    _spread(fp, qs[1:1 + len(fp)])
                else:
                    if sm is not None:
                        stg += [[] for _ in range(100 - len(stg))]
                    _spread(fp, stg)
            l = [None] * NQ
            shifts = []
            ns = 0
            if qk is not None:
                for hh in range(NQ):
                    ws = weights(qk[0], qk[1], hh)
                    ts = []
                    for ci in range(NC):
                        clock[0] += 1
                        t, m3 = trio(ws, sbufs[qk[2]], ci, hh)
                        ts.append(t)
                        if swap_a and hh == NQ - 1:
                            rows = pl.ds(ci * R // 2, R // 2)
                            a_scr[:, rows, :] = an_scr[:, rows, :]
                        while pend and loads[3] < loads[0]:
                            pend.pop(0)(None)
                        l = sm_slab(sm, ns, m_sm, l, [m3[i * 24:i * 24 + 8] for i in range(4)])
                        y_fence(sm, l, YLAG)
                        for n, piece in enumerate(qs[ns]):
                            r0 = 112 if len(qs[ns]) == 1 else (n * 112 // (len(qs[ns]) - 1)) // 8 * 8
                            piece(m3[r0:r0 + 16])
                        ns += 1
                    shifts.append(row_shift(ts))
            if mid is not None:
                mid()
            n = 0
            recent = []
            while pend:
                if (not final and len(pend) <= 3
                        and loads[0] == loads[1] == loads[2] and loads[3] >= loads[0]):
                    break
                if n % 4 == 0:
                    clock[0] += 1
                n += 1
                tile = pend.pop(0)
                o = tile(take_fences(flush=(final and len(pend) == 1)), final == 2 and not pend)
                if stg:
                    for piece in stg.pop(0):
                        piece(o)
                if sm is not None and ns < NG * SPG:
                    recent.append(o)
                    if len(recent) == 3:
                        l = sm_slab(sm, ns, m_sm, l,
                                    [recent[0][0:8], recent[1][16:24], recent[2][32:40], recent[2][56:64]])
                        ns += 1
                        recent = []
                        y_fence(sm, l, ELAG)
            assert not any(stg) and (sm is None or ns == NG * SPG)
            return (tuple(shifts) if qk is not None else None), (tuple(l) if sm is not None else None), l_pv

        vall = [(g, rb, e) for g in range(NG) for rb in range(NRB) for e in range(7)]
        nv = len(vall) // 3

        def q0_copy(a, b, sem):
            cs = pl.ds(a * W, (b - a) * W)
            return pltpu.make_async_copy(q_hbm.at[0, :, cs], qb.at[0, :, cs], p_sem.at[sem])

        def k0_copy(hf, sem):
            cs = pl.ds(hf * half, half)
            return pltpu.make_async_copy(k_hbm.at[0, :, cs], kb.at[0, pl.ds(0, D), cs], p_sem.at[sem])

        ck0a, ck0b = k0_copy(0, 0), k0_copy(1, 1)
        cq0, cq1, cq2 = q0_copy(0, 1, 2), q0_copy(1, 2, 3), q0_copy(2, 4, 4)
        for cp in (ck0a, cq0, ck0b, v_copy(0, 0), cq1, cq2, k_copy(1, 1), v_copy(1, 1)):
            cp.start()
        small = lax.fori_loop(0, 3, lambda i, acc: acc + i, jnp.int32(0))
        ck0a.wait()
        cq0.wait()
        new_block(small)
        wss = [weights(0, 0, hh) for hh in range(NQ)]
        tss = [[] for _ in range(NQ)]
        v0 = sorted(vall, key=lambda x: x[2])
        qs0 = [[] for _ in range(NC * NQ // 2)]
        _spread(v_pieces(0, v0[:96], x_scr), qs0)
        for ci in range(NC):
            if ci == NC // 2:
                ck0b.wait()
                v_copy(0, 0).wait()
                cq1.wait()
                new_block(small)
            kprep(0, ci, a_scr)
            for hh in range(NQ):
                clock[0] += 1
                t, m3 = trio(wss[hh], sbufs[0], ci, hh)
                tss[hh].append(t)
                if ci >= NC // 2:
                    for n, piece in enumerate(qs0.pop(0)):
                        piece(m3[(n * 24) % 112:(n * 24) % 112 + 16])
        st = (tuple(row_shift(t) for t in tss), None, None)
        st = step((0, 1, 1), 0, None, None, st)
        cq2.wait()
        k_copy(1, 1).wait()
        v_copy(1, 1).wait()
        q_copy(1, 1).start()
        k_copy(2, 0).start()
        new_block(small)
        st = step((0, 2, 0), 1, 0, None, st, final=2, stg=stage(1, range(NC), 1, vall[:nv], 6),
                  qx=v_pieces(0, v0[96:], x_scr), mid=lambda: v_copy(2, 0).start())

        def head(h, st):
            cur = h & 1
            nx = 1 - cur
            new_block(h)
            q_copy(0, nx).wait()
            k_copy(0, cur).wait()
            v_copy(0, cur).wait()

            @pl.when(h > 1)
            def _():
                out_copy(h - 2, cur).wait()

            @pl.when(h > 0)
            def _():
                out_copy(h - 1, nx).start()

            k_copy(jnp.minimum(h + 3, H - 1), nx).start()
            add_fence(3, _bits(kb[cur, zrows(0, 8, 16), 0:R].astype(f32)))
            st = step((cur, 3, 1), 0, 1, (cur, 0, 0), st, swap_a=True,
                      stg=stage(cur, [0, 1], nx, vall[nv:2 * nv]))
            q_copy(jnp.minimum(h + 2, H - 1), cur).start()
            st = step((nx, 0, 0), 1, 0, (cur, 1, 1), st, stg=stage(cur, [2, 3], nx, vall[2 * nv:]))
            v_copy(jnp.minimum(h + 3, H - 1), nx).start()
            add_fence(12, _bits(vb[cur, zrows(0, 8, 16), 0:R].astype(f32)))
            st = step((nx, 1, 1), 0, 1, (cur, 2, 0), st, swap_x=True, stg=stage(cur, [4, 5, 6, 7], nx, []))
            return step((nx, 2, 0), 1, 0, (cur, 3, 1), st, final=2, stg=stage(cur, [], cur, vall[:nv]))

        st = lax.fori_loop(0, H - 1, head, st)

        last = (H - 1) % 2
        new_block(small)

        def last_copy(a, b, sem):
            cs = pl.ds(a * W, (b - a) * W)
            return pltpu.make_async_copy(outb.at[last, :, cs], o_hbm.at[H - 1, :, cs], p_sem.at[sem])

        e1, e2 = last_copy(0, 3, 1), last_copy(3, 4, 2)
        out_copy(H - 3, last).wait()
        out_copy(H - 2, 1 - last).start()
        st = step((last, 3, 1), 0, 1, (last, 0, 0), st, final=1)
        st = step(None, 1, 0, (last, 1, 1), st, final=1)
        st = step(None, None, 1, (last, 2, 0), st, final=1)
        e1.start()
        step(None, None, None, (last, 3, 1), st, final=1)
        e2.start()
        q_copy(0, 1 - last).wait()
        k_copy(0, last).wait()
        v_copy(0, last).wait()
        out_copy(H - 2, 1 - last).wait()
        e1.wait()
        e2.wait()

    ot = pl.pallas_call(
        body,
        in_specs=[pl.BlockSpec(memory_space=pl.ANY)] * 3,
        out_specs=pl.BlockSpec(memory_space=pl.ANY),
        out_shape=jax.ShapeDtypeStruct((H, D, S), bf16),
        scratch_shapes=[
            pltpu.VMEM((2, D, S), bf16),
            pltpu.VMEM((2, D + 16, S), bf16),
            pltpu.VMEM((2, D + 16, S), bf16),
            pltpu.VMEM((2, D, S), bf16),
            pltpu.VMEM((3, half // 2, R), u32),
            pltpu.VMEM((NP, NG, hd // 2, R), u32),
            pltpu.VMEM((3, half // 2, R), u32),
            pltpu.VMEM((NP + 1, NG, hd // 2, R), u32),
            pltpu.VMEM((NQ, 2 * NC, R, R), f32),
            pltpu.VMEM((NQ, 2 * NC, R, R), f32),
            pltpu.VMEM((NP, NG * R + 16, R), bf16),
            pltpu.VMEM((NP, NG * R + 16, R), bf16),
            pltpu.VMEM((NP + 1, hd, R), f32),
            pltpu.VMEM((NP + 1, hd, R), f32),
            pltpu.SemaphoreType.DMA((2,)),
            pltpu.SemaphoreType.DMA((2,)),
            pltpu.SemaphoreType.DMA((2,)),
            pltpu.SemaphoreType.DMA((2,)),
            pltpu.SemaphoreType.DMA((5,)),
        ],
        compiler_params=pltpu.CompilerParams(vmem_limit_bytes=100 * 1024 * 1024),
    )(qt, kt, vt)
    return jnp.swapaxes(ot.reshape(B, NH, D, S), 2, 3)
```

```python
import itertools
import math

import jax
import jax.numpy as jnp
from jax import lax
import jax.experimental.pallas as pl
import jax.experimental.pallas.tpu as pltpu

f32 = jnp.float32
bf16 = jnp.bfloat16
i32 = jnp.int32
u32 = jnp.uint32

W = 512
R = 128
SLAB = 16
NP = 26
T = (-1.375, -0.328125, 0.328125, 1.375)
PAIRS = tuple(itertools.combinations(range(4), 2))
BS = {(0, 1): 1.0, (0, 2): 1.0, (0, 3): -1.0, (1, 2): -1.0, (1, 3): 1.0, (2, 3): 1.0}
YLAG, SLAG, KLAG, CLAG, ELAG, NST = 6, 5, 9, 4, 3, 52


def _tree(parts, op):
    parts = list(parts)
    while len(parts) > 1:
        nxt = [op(parts[i], parts[i + 1]) for i in range(0, len(parts) - 1, 2)]
        if len(parts) % 2:
            nxt.append(parts[-1])
        parts = nxt
    return parts[0]


def _bits(x):
    return lax.bitcast_convert_type(x, i32)


def _spread(pieces, slots):
    for n, piece in enumerate(pieces):
        slots[n * len(slots) // len(pieces)].append(piece)


@jax.jit
def pallas_standalone__mha_softmax__prompt_kernel(q: jax.Array, k: jax.Array, v: jax.Array):
    B, NH, S, D = q.shape
    H = B * NH
    assert D == 192 and S == 2048 and H >= 3 and k.shape == q.shape and v.shape == q.shape
    qt = jnp.swapaxes(q, 2, 3).reshape(H, D, S)
    kt = jnp.swapaxes(k, 2, 3).reshape(H, D, S)
    vt = jnp.swapaxes(v, 2, 3).reshape(H, D, S)
    c = (D ** -0.5) * math.log2(math.e)
    hd = D // 2
    half = S // 2
    NC = S // (2 * R)
    NG = S // (4 * R)
    NQ = W // R
    SPG = R // SLAB
    NRB = hd // 16

    def body(q_hbm, k_hbm, v_hbm, o_hbm, qb, kb, vb, outb, a_scr, x_scr, an_scr, xn_scr,
             s0, s1, y0, y1, m0, m1, q_sem, k_sem, v_sem, out_sem, p_sem):
        sbufs = (s0, s1)
        ybufs = (y0, y1)
        mbufs = (m0, m1)
        zero = {}
        fences = []
        clock = [0]
        loads = [0, 0, 0, 0]
        pend = []

        def new_block(i):
            zero.clear()
            zero["s"] = lax.shift_right_logical(i, 16)
            zero["v"] = jnp.full((8, R), zero["s"], i32)
            fences.clear()
            loads[:] = [0, 0, 0, 0]

        def zrows(base=0, n=8, align=8):
            if (base, align) not in zero:
                zero[(base, align)] = pl.multiple_of(base + zero["s"] * align, align)
            return pl.ds(zero[(base, align)], n)

        def add_fence(lag, tok):
            fences.append((clock[0] + lag, tok, clock[0]))

        def take_fences(flush=False):
            def ok(x):
                return x[0] <= clock[0] or (flush and x[2] + 3 <= clock[0])
            due = [x[1] for x in fences if ok(x)]
            fences[:] = [x for x in fences if not ok(x)]
            if not due:
                return None
            return lax.bitcast_convert_type(_tree(due, jnp.bitwise_or) & zero["v"], u32)

        def lhs(a, tok):
            if tok is not None:
                a = jnp.concatenate([a[0:8] | tok, a[8:]], axis=0)
            return pltpu.bitcast(a, bf16)

        def q_copy(h, slot):
            return pltpu.make_async_copy(q_hbm.at[h], qb.at[slot], q_sem.at[slot])

        def k_copy(h, slot):
            return pltpu.make_async_copy(k_hbm.at[h], kb.at[slot, pl.ds(0, D)], k_sem.at[slot])

        def v_copy(h, slot):
            return pltpu.make_async_copy(v_hbm.at[h], vb.at[slot, pl.ds(0, D)], v_sem.at[slot])

        def out_copy(h, slot):
            return pltpu.make_async_copy(outb.at[slot], o_hbm.at[h], out_sem.at[slot])

        def kprep(slot, ci, dst):
            k1 = kb[slot, 0:D, pl.ds(2 * ci * R, R)].astype(f32)
            k2 = kb[slot, 0:D, pl.ds(2 * ci * R + R, R)].astype(f32)
            a1t = jnp.concatenate([k1[0:64], k1[64:128] - k2[64:128]], axis=0)
            a2t = jnp.concatenate([k2[0:64], k2[128:192] - k1[128:192]], axis=0)
            a3t = jnp.concatenate([k2[64:128], k1[128:192]], axis=0)
            for i, x in enumerate((a1t, a2t, a3t)):
                dst[i, pl.ds(ci * (R // 2), R // 2), :] = pltpu.bitcast(x.T.astype(bf16), u32)

        def vprep(slot, g, rb, e, dst):
            def blk(rr, kk):
                return vb[slot, pl.ds(rr * hd + rb * 16, 16), pl.ds((4 * g + kk) * R, R)]

            def put(r, x):
                dst[r, g, pl.ds(rb * 8, 8), :] = pltpu.bitcast(x.astype(bf16), u32)

            if e == 6:
                for kk in range(4):
                    lo = blk(1, kk)
                    put(18 + 2 * kk, blk(0, kk).astype(f32) + T[kk] * lo.astype(f32))
                    put(19 + 2 * kk, lo)
                return
            kk, qq = PAIRS[e]
            b = BS[(kk, qq)]
            it = 1.0 / (T[qq] - T[kk])
            u1k = blk(0, kk).astype(f32)
            u2k = blk(1, kk).astype(f32)
            u1q = blk(0, qq).astype(f32)
            u2q = blk(1, qq).astype(f32)
            top = ((u1k + u1q) if b > 0 else (u1k - u1q)) * it
            xa = top + u2k * (T[qq] * it) + u2q * (b * T[qq] * it)
            put(3 * e, xa)
            xc = xa - u2k
            put(3 * e + 2, xc)
            put(3 * e + 1, (xc - u2q) if b > 0 else (xc + u2q))

        def k_piece(slot, ci):
            def f(anchor):
                kb[slot, zrows(D, 16, 16), 0:R] = anchor[0:16].astype(bf16)
                kprep(slot, ci, an_scr)
                add_fence(KLAG, _bits(an_scr[0, zrows(ci * (R // 2)), :]))
            return f

        def v_pieces(slot, vps, dst):
            def mk(g, rb, e, fence):
                def f(anchor):
                    vb[slot, zrows(D, 16, 16), 0:R] = anchor[0:16].astype(bf16)
                    vprep(slot, g, rb, e, dst)
                    if fence:
                        add_fence(KLAG, _bits(dst[3 * e, g, zrows(rb * 8), :]))
                return f
            return [mk(g, rb, e, n % 4 == 3 or n == len(vps) - 1) for n, (g, rb, e) in enumerate(vps)]

        def stage(kslot, kcs, vslot, vps, kgap=12):
            out = [[] for _ in range(NST)]
            for n, ci in enumerate(kcs):
                out[n * kgap].append(k_piece(kslot, ci))
            _spread(v_pieces(vslot, vps, xn_scr), out)
            return out

        def weights(slot, u, hh):
            qc = qb[slot, :, pl.ds(u * W + hh * R, R)]
            return (qc[0:128], jnp.concatenate([qc[0:64], qc[128:192]], axis=0), qc[64:192])

        def trio(ws, s_ref, ci, hh):
            rows = pl.ds(ci * R // 2, R // 2)
            tok = take_fences()
            m3 = jnp.dot(lhs(a_scr[2, rows, :], tok), ws[2], preferred_element_type=f32)
            m1 = jnp.dot(lhs(a_scr[0, rows, :], tok), ws[0], preferred_element_type=f32)
            m2 = jnp.dot(lhs(a_scr[1, rows, :], tok), ws[1], preferred_element_type=f32)
            for _ in range(3):
                loads[loads.index(min(loads))] += R
            sa = (m1 + m3) * c
            sb = (m2 + m3) * c
            s_ref[hh, 2 * ci] = sa
            s_ref[hh, 2 * ci + 1] = sb
            t = jnp.maximum(sa, sb).reshape(R // 8, 8, R).max(axis=0)
            add_fence(SLAG, _bits(s_ref[0, 0, zrows(), :]) | _bits(t))
            return t, m3

        def row_shift(ts):
            m = jnp.max(_tree(ts, jnp.maximum), axis=0, keepdims=True)
            n2 = jnp.sum(_tree([jnp.exp2((t - m) * 2.0) for t in ts], jnp.add), axis=0, keepdims=True)
            return _bits(jnp.broadcast_to(m + jnp.log2(n2) * 0.5, (8, R)))

        def sm_slab(par, idx, m8, l, anchors):
            g, b = divmod(idx, SPG)
            rows = pl.ds(b * SLAB, SLAB)
            yrows = pl.ds(g * R + b * SLAB, SLAB)

            def mk_exp(anchor, qs):
                tk = _bits(anchor) & zero["v"]
                mm = {qq: lax.bitcast_convert_type(m8[qq] | tk, f32) for qq in qs}
                mm = {qq: jnp.concatenate([x, x], axis=0) for qq, x in mm.items()}
                return lambda kk, qq: jnp.exp2(sbufs[par][qq, 4 * g + kk, rows, :] - mm[qq])

            def put(r, x):
                ybufs[par][r, yrows, :] = x.astype(bf16)

            def diff(kk, qq, pkq, pqk):
                put(3 * PAIRS.index((kk, qq)) + 2, pkq - pqk)

            def single(kk, qq, p):
                if kk < qq:
                    put(3 * PAIRS.index((kk, qq)), p)
                else:
                    put(3 * PAIRS.index((qq, kk)) + 1, p)

            uc = {}
            ur = {}
            for n, (i, j) in enumerate(((0, 3), (1, 2))):
                ex = mk_exp(anchors[n], (i, j))
                pii, pjj, pij, pji = ex(i, i), ex(j, j), ex(i, j), ex(j, i)
                single(i, j, pij)
                single(j, i, pji)
                diff(i, j, pij, pji)
                uc[i] = pii + pji
                uc[j] = pjj + pij
                ur[i] = pii + pij
                ur[j] = pjj + pji
            keep = {}
            l = list(l)
            for n, (rs, cs) in enumerate((((0, 3), (1, 2)), ((1, 2), (0, 3)))):
                ex = mk_exp(anchors[2 + n], cs)
                p = {(kk, qq): ex(kk, qq) for kk in rs for qq in cs}
                for (kk, qq), x in p.items():
                    single(kk, qq, x)
                for kk in rs:
                    put(19 + 2 * kk, ur[kk] - (p[(kk, cs[0])] + p[(kk, cs[1])]))
                for qq in cs:
                    vc = p[(rs[0], qq)] + p[(rs[1], qq)]
                    put(18 + 2 * qq, uc[qq] - vc)
                    tot = uc[qq] + vc
                    tot = tot[0:8] + tot[8:16]
                    l[qq] = tot if l[qq] is None else l[qq] + tot
                if n == 0:
                    keep = p
                else:
                    for (kk, qq), x in p.items():
                        if kk < qq:
                            diff(kk, qq, x, keep[(qq, kk)])
                        else:
                            diff(qq, kk, keep[(qq, kk)], x)
            return l

        def y_fence(par, l, lag):
            tok = _bits(ybufs[par][0, zrows(0, 8, 16), :].astype(f32))
            add_fence(lag, _tree([tok] + [_bits(x) for x in l], jnp.bitwise_or))

        def queue_pv(par, swap_x):
            ms = {}

            def mk(i, j):
                def f(tok, even=False):
                    yy = pltpu.bitcast(ybufs[par].bitcast(u32)[i, pl.ds(j * R // 2, R // 2), :], bf16)
                    xx = lhs(x_scr[i, j], tok)
                    if even:
                        assert loads[0] == loads[1] == loads[2] == loads[3] - hd // 3
                        o = jnp.concatenate(
                            [jnp.dot(xx[a:a + hd // 3], yy, preferred_element_type=f32)
                             for a in range(0, hd, hd // 3)], axis=0)
                    else:
                        o = jnp.dot(xx, yy, preferred_element_type=f32)
                    ms[i] = o if j == 0 else ms[i] + o
                    loads[loads.index(min(loads))] += hd
                    if swap_x and j % 2 == 1:
                        xn_scr[NP, 0, zrows(), :] = lax.bitcast_convert_type(o[0:8], u32)
                        for jj in (j - 1, j):
                            x_scr[i, jj] = xn_scr[i, jj]
                    if j == NG - 1:
                        mbufs[par][i] = ms[i]
                        add_fence(CLAG, _bits(mbufs[par][i, zrows(), :]))
                    return o
                return f

            for i in range(NP):
                for j in range(NG):
                    pend.append(mk(i, j))

        def fin_pieces(fin, l_fin):
            slot, u, par = fin
            m_ref = mbufs[par]
            rls = {}

            def mk(qq, rb):
                def f(anchor):
                    if anchor is not None:
                        m_ref[NP, zrows(), :] = anchor[0:8]
                    if qq not in rls:
                        rls[qq] = 1.0 / jnp.sum(l_fin[qq], axis=0, keepdims=True)

                    def prod(r):
                        return m_ref[r, pl.ds(rb * 16, 16), :]

                    gq = prod(19 + 2 * qq)
                    oth = []
                    for e, (i, j) in enumerate(PAIRS):
                        b = BS[(i, j)]
                        if qq == j:
                            oth.append((i, prod(3 * e), 1.0))
                            gq = gq - (prod(3 * e + 1) + prod(3 * e + 2))
                        elif qq == i:
                            d = prod(3 * e) - prod(3 * e + 2)
                            gq = (gq + d) if b > 0 else (gq - d)
                            oth.append((j, prod(3 * e + 1), -b))
                    c1 = prod(18 + 2 * qq) - gq * T[qq]
                    c2 = gq
                    for kk, gv, sg in oth:
                        c1 = c1 - gv * (T[kk] * sg)
                        c2 = (c2 + gv) if sg > 0 else (c2 - gv)
                    cols = pl.ds(u * W + qq * R, R)
                    outb[slot, pl.ds(rb * 16, 16), cols] = (c1 * rls[qq]).astype(bf16)
                    outb[slot, pl.ds(hd + rb * 16, 16), cols] = (c2 * rls[qq]).astype(bf16)
                    if anchor is not None and rb % 3 == 2:
                        add_fence(KLAG, _bits(outb[slot, zrows(rb * 16, 8, 16), cols].astype(f32)))
                return f
            return [mk(qq, rb) for qq in range(NQ) for rb in range(NRB)]

        def step(qk, sm, pv, fin, st, swap_a=False, swap_x=False, final=0, stg=None, qx=(), mid=None):
            m_sm, l_pv, l_fin = st
            if pv is not None:
                queue_pv(pv, swap_x)
            stg = stg or [[] for _ in range(NST)]
            qs = [[] for _ in range(NQ * NC)]
            _spread(list(qx), qs[:NQ * NC - 2])
            if fin is not None:
                fp = fin_pieces(fin, l_fin)
                if pv is None:
                    for piece in fp:
                        piece(None)
                elif qk is not None:
                    _spread(fp, qs[1:1 + len(fp)])
                else:
                    if sm is not None:
                        stg += [[] for _ in range(100 - len(stg))]
                    _spread(fp, stg)
            l = [None] * NQ
            shifts = []
            ns = 0
            if qk is not None:
                for hh in range(NQ):
                    ws = weights(qk[0], qk[1], hh)
                    ts = []
                    for ci in range(NC):
                        clock[0] += 1
                        t, m3 = trio(ws, sbufs[qk[2]], ci, hh)
                        ts.append(t)
                        if swap_a and hh == NQ - 1:
                            rows = pl.ds(ci * R // 2, R // 2)
                            a_scr[:, rows, :] = an_scr[:, rows, :]
                        while pend and loads[3] < loads[0]:
                            pend.pop(0)(None)
                        l = sm_slab(sm, ns, m_sm, l, [m3[i * 24:i * 24 + 8] for i in range(4)])
                        y_fence(sm, l, YLAG)
                        for n, piece in enumerate(qs[ns]):
                            r0 = 112 if len(qs[ns]) == 1 else (n * 112 // (len(qs[ns]) - 1)) // 8 * 8
                            piece(m3[r0:r0 + 16])
                        ns += 1
                    shifts.append(row_shift(ts))
            if mid is not None:
                mid()
            n = 0
            recent = []
            while pend:
                if (not final and len(pend) <= 3
                        and loads[0] == loads[1] == loads[2] and loads[3] >= loads[0]):
                    break
                if n % 4 == 0:
                    clock[0] += 1
                n += 1
                tile = pend.pop(0)
                o = tile(take_fences(flush=(final and len(pend) == 1)), final == 2 and not pend)
                if stg:
                    for piece in stg.pop(0):
                        piece(o)
                if sm is not None and ns < NG * SPG:
                    recent.append(o)
                    if len(recent) == 3:
                        l = sm_slab(sm, ns, m_sm, l,
                                    [recent[0][0:8], recent[1][16:24], recent[2][32:40], recent[2][56:64]])
                        ns += 1
                        recent = []
                        y_fence(sm, l, ELAG)
            assert not any(stg) and (sm is None or ns == NG * SPG)
            return (tuple(shifts) if qk is not None else None), (tuple(l) if sm is not None else None), l_pv

        vall = [(g, rb, e) for g in range(NG) for rb in range(NRB) for e in range(7)]
        nv = len(vall) // 3

        def q0_copy(a, b, sem):
            cs = pl.ds(a * W, (b - a) * W)
            return pltpu.make_async_copy(q_hbm.at[0, :, cs], qb.at[0, :, cs], p_sem.at[sem])

        def k0_copy(hf, sem):
            cs = pl.ds(hf * half, half)
            return pltpu.make_async_copy(k_hbm.at[0, :, cs], kb.at[0, pl.ds(0, D), cs], p_sem.at[sem])

        ck0a, ck0b = k0_copy(0, 0), k0_copy(1, 1)
        cq0, cq1, cq2 = q0_copy(0, 1, 2), q0_copy(1, 2, 3), q0_copy(2, 4, 4)
        for cp in (ck0a, cq0, ck0b, v_copy(0, 0), cq1, cq2, k_copy(1, 1), v_copy(1, 1)):
            cp.start()
        small = lax.fori_loop(0, 3, lambda i, acc: acc + i, jnp.int32(0))
        ck0a.wait()
        cq0.wait()
        new_block(small)
        wss = [weights(0, 0, hh) for hh in range(NQ)]
        tss = [[] for _ in range(NQ)]
        v0 = sorted(vall, key=lambda x: x[2])
        qs0 = [[] for _ in range(NC * NQ // 2)]
        _spread(v_pieces(0, v0[:96], x_scr), qs0)
        for ci in range(NC):
            if ci == NC // 2:
                ck0b.wait()
                v_copy(0, 0).wait()
                cq1.wait()
                new_block(small)
            kprep(0, ci, a_scr)
            for hh in range(NQ):
                clock[0] += 1
                t, m3 = trio(wss[hh], sbufs[0], ci, hh)
                tss[hh].append(t)
                if ci >= NC // 2:
                    for n, piece in enumerate(qs0.pop(0)):
                        piece(m3[(n * 24) % 112:(n * 24) % 112 + 16])
        st = (tuple(row_shift(t) for t in tss), None, None)
        st = step((0, 1, 1), 0, None, None, st)
        cq2.wait()
        k_copy(1, 1).wait()
        v_copy(1, 1).wait()
        q_copy(1, 1).start()
        k_copy(2, 0).start()
        new_block(small)
        st = step((0, 2, 0), 1, 0, None, st, final=2, stg=stage(1, range(NC), 1, vall[:nv], 6),
                  qx=v_pieces(0, v0[96:], x_scr), mid=lambda: v_copy(2, 0).start())

        def head(h, st):
            cur = h & 1
            nx = 1 - cur
            new_block(h)
            q_copy(0, nx).wait()
            k_copy(0, cur).wait()
            v_copy(0, cur).wait()

            @pl.when(h > 1)
            def _():
                out_copy(h - 2, cur).wait()

            @pl.when(h > 0)
            def _():
                out_copy(h - 1, nx).start()

            k_copy(jnp.minimum(h + 3, H - 1), nx).start()
            add_fence(3, _bits(kb[cur, zrows(0, 8, 16), 0:R].astype(f32)))
            st = step((cur, 3, 1), 0, 1, (cur, 0, 0), st, swap_a=True,
                      stg=stage(cur, [0, 1], nx, vall[nv:2 * nv]))
            q_copy(jnp.minimum(h + 2, H - 1), cur).start()
            st = step((nx, 0, 0), 1, 0, (cur, 1, 1), st, stg=stage(cur, [2, 3], nx, vall[2 * nv:]))
            v_copy(jnp.minimum(h + 3, H - 1), nx).start()
            add_fence(12, _bits(vb[cur, zrows(0, 8, 16), 0:R].astype(f32)))
            st = step((nx, 1, 1), 0, 1, (cur, 2, 0), st, swap_x=True, stg=stage(cur, [4, 5, 6, 7], nx, []))
            return step((nx, 2, 0), 1, 0, (cur, 3, 1), st, final=2, stg=stage(cur, [], cur, vall[:nv]))

        st = lax.fori_loop(0, H - 1, head, st)

        last = (H - 1) % 2
        new_block(small)

        def last_copy(a, b, sem):
            cs = pl.ds(a * W, (b - a) * W)
            return pltpu.make_async_copy(outb.at[last, :, cs], o_hbm.at[H - 1, :, cs], p_sem.at[sem])

        e1, e2 = last_copy(0, 3, 1), last_copy(3, 4, 2)
        out_copy(H - 3, last).wait()
        out_copy(H - 2, 1 - last).start()
        st = step((last, 3, 1), 0, 1, (last, 0, 0), st, final=1)
        st = step(None, 1, 0, (last, 1, 1), st, final=1)
        st = step(None, None, 1, (last, 2, 0), st, final=1)
        e1.start()
        step(None, None, None, (last, 3, 1), st, final=1)
        e2.start()
        q_copy(0, 1 - last).wait()
        k_copy(0, last).wait()
        v_copy(0, last).wait()
        out_copy(H - 2, 1 - last).wait()
        e1.wait()
        e2.wait()

    ot = pl.pallas_call(
        body,
        in_specs=[pl.BlockSpec(memory_space=pl.ANY)] * 3,
        out_specs=pl.BlockSpec(memory_space=pl.ANY),
        out_shape=jax.ShapeDtypeStruct((H, D, S), bf16),
        scratch_shapes=[
            pltpu.VMEM((2, D, S), bf16),
            pltpu.VMEM((2, D + 16, S), bf16),
            pltpu.VMEM((2, D + 16, S), bf16),
            pltpu.VMEM((2, D, S), bf16),
            pltpu.VMEM((3, half // 2, R), u32),
            pltpu.VMEM((NP, NG, hd // 2, R), u32),
            pltpu.VMEM((3, half // 2, R), u32),
            pltpu.VMEM((NP + 1, NG, hd // 2, R), u32),
            pltpu.VMEM((NQ, 2 * NC, R, R), f32),
            pltpu.VMEM((NQ, 2 * NC, R, R), f32),
            pltpu.VMEM((NP, NG * R + 16, R), bf16),
            pltpu.VMEM((NP, NG * R + 16, R), bf16),
            pltpu.VMEM((NP + 1, hd, R), f32),
            pltpu.VMEM((NP + 1, hd, R), f32),
            pltpu.SemaphoreType.DMA((2,)),
            pltpu.SemaphoreType.DMA((2,)),
            pltpu.SemaphoreType.DMA((2,)),
            pltpu.SemaphoreType.DMA((2,)),
            pltpu.SemaphoreType.DMA((5,)),
        ],
        compiler_params=pltpu.CompilerParams(vmem_limit_bytes=100 * 1024 * 1024),
    )(qt, kt, vt)
    return jnp.swapaxes(ot.reshape(B, NH, D, S), 2, 3)
```

```python
import itertools
import math

import jax
import jax.numpy as jnp
from jax import lax
import jax.experimental.pallas as pl
import jax.experimental.pallas.tpu as pltpu

f32 = jnp.float32
bf16 = jnp.bfloat16
i32 = jnp.int32
u32 = jnp.uint32

W = 512
R = 128
SLAB = 16
NP = 26
T = (-1.375, -0.328125, 0.328125, 1.375)
PAIRS = tuple(itertools.combinations(range(4), 2))
BS = {(0, 1): 1.0, (0, 2): 1.0, (0, 3): -1.0, (1, 2): -1.0, (1, 3): 1.0, (2, 3): 1.0}
YLAG, SLAG, KLAG, CLAG, ELAG, NST = 5, 4, 9, 4, 3, 52


def _tree(parts, op):
    parts = list(parts)
    while len(parts) > 1:
        nxt = [op(parts[i], parts[i + 1]) for i in range(0, len(parts) - 1, 2)]
        if len(parts) % 2:
            nxt.append(parts[-1])
        parts = nxt
    return parts[0]


def _bits(x):
    return lax.bitcast_convert_type(x, i32)


def _spread(pieces, slots):
    for n, piece in enumerate(pieces):
        slots[n * len(slots) // len(pieces)].append(piece)


@jax.jit
def pallas_standalone__mha_softmax__prompt_kernel(q: jax.Array, k: jax.Array, v: jax.Array):
    B, NH, S, D = q.shape
    H = B * NH
    assert D == 192 and S == 2048 and H >= 3 and k.shape == q.shape and v.shape == q.shape
    qt = jnp.swapaxes(q, 2, 3).reshape(H, D, S)
    kt = jnp.swapaxes(k, 2, 3).reshape(H, D, S)
    vt = jnp.swapaxes(v, 2, 3).reshape(H, D, S)
    c = (D ** -0.5) * math.log2(math.e)
    hd = D // 2
    half = S // 2
    NC = S // (2 * R)
    NG = S // (4 * R)
    NQ = W // R
    SPG = R // SLAB
    NRB = hd // 16

    def body(q_hbm, k_hbm, v_hbm, o_hbm, qb, kb, vb, outb, a_scr, x_w, an_scr, xn_w,
             s0, s1, y0, y1, m0, m1, mu_scr, q_sem, k_sem, v_sem, out_sem, p_sem):
        sbufs = (s0, s1)
        ybufs = (y0, y1)
        mbufs = (m0, m1)
        x_scr = x_w.bitcast(u32)
        xn_scr = xn_w.bitcast(u32)
        zero = {}
        fences = []
        clock = [0]
        loads = [0, 0, 0, 0]
        pend = []

        def new_block(i):
            zero.clear()
            zero["s"] = lax.shift_right_logical(i, 16)
            zero["v"] = jnp.full((8, R), zero["s"], i32)
            fences.clear()
            loads[:] = [0, 0, 0, 0]

        def zrows(base=0, n=8, align=8):
            if (base, align) not in zero:
                zero[(base, align)] = pl.multiple_of(base + zero["s"] * align, align)
            return pl.ds(zero[(base, align)], n)

        def add_fence(lag, tok):
            fences.append((clock[0] + lag, tok, clock[0]))

        def take_fences(flush=False):
            def ok(x):
                return x[0] <= clock[0] or (flush and x[2] + 3 <= clock[0])
            due = [x[1] for x in fences if ok(x)]
            fences[:] = [x for x in fences if not ok(x)]
            if not due:
                return None
            return lax.bitcast_convert_type(_tree(due, jnp.bitwise_or) & zero["v"], u32)

        def lhs(a, tok):
            if tok is not None:
                a = jnp.concatenate([a[0:8] | tok, a[8:]], axis=0)
            return pltpu.bitcast(a, bf16)

        def q_copy(h, slot):
            return pltpu.make_async_copy(q_hbm.at[h], qb.at[slot], q_sem.at[slot])

        def k_copy(h, slot):
            return pltpu.make_async_copy(k_hbm.at[h], kb.at[slot, pl.ds(0, D)], k_sem.at[slot])

        def v_copy(h, slot):
            return pltpu.make_async_copy(v_hbm.at[h], vb.at[slot, pl.ds(0, D)], v_sem.at[slot])

        def out_copy(h, slot):
            return pltpu.make_async_copy(outb.at[slot], o_hbm.at[h], out_sem.at[slot])

        def kprep(slot, ci, dst):
            k1 = kb[slot, 0:D, pl.ds(2 * ci * R, R)].astype(f32)
            k2 = kb[slot, 0:D, pl.ds(2 * ci * R + R, R)].astype(f32)
            a1t = jnp.concatenate([k1[0:64], k1[64:128] - k2[64:128]], axis=0)
            a2t = jnp.concatenate([k2[0:64], k2[128:192] - k1[128:192]], axis=0)
            a3t = jnp.concatenate([k2[64:128], k1[128:192]], axis=0)
            for i, x in enumerate((a1t, a2t, a3t)):
                dst[i, pl.ds(ci * (R // 2), R // 2), :] = pltpu.bitcast(x.T.astype(bf16), u32)

        def mu_piece(slot, ms):
            def f(anchor):
                if anchor is not None:
                    vb[slot, zrows(D, 16, 16), 0:R] = anchor[0:16].astype(bf16)
                x = vb[slot, 0:D, 0:R].astype(f32)
                mu_scr[ms] = jnp.broadcast_to(jnp.sum(x, axis=1, keepdims=True) * (1.0 / R), (D, R))
            return f

        def vprep(slot, ms, g, rb, e, dst):
            def blk(rr, kk):
                return vb[slot, pl.ds(rr * hd + rb * 16, 16), pl.ds((4 * g + kk) * R, R)].astype(f32)

            def put(r, x):
                dst[r, g, pl.ds(rb * 16, 16), :] = x.astype(bf16)

            mu1 = mu_scr[ms, pl.ds(rb * 16, 16), :]
            mu2 = mu_scr[ms, pl.ds(hd + rb * 16, 16), :]
            if e == 6:
                for kk in range(4):
                    lo = blk(1, kk) - mu2
                    put(18 + 2 * kk, (blk(0, kk) - mu1) + T[kk] * lo)
                    put(19 + 2 * kk, lo)
                return
            kk, qq = PAIRS[e]
            b = BS[(kk, qq)]
            it = 1.0 / (T[qq] - T[kk])
            u2k = blk(1, kk) - mu2
            u2q = blk(1, qq) - mu2
            top = ((blk(0, kk) - mu1) + (blk(0, qq) - mu1)) if b > 0 else (blk(0, kk) - blk(0, qq))
            xa = top * it + ((u2k + u2q) if b > 0 else (u2k - u2q)) * (T[qq] * it)
            put(3 * e, xa)
            xc = xa - u2k
            put(3 * e + 2, xc)
            put(3 * e + 1, (xc - u2q) if b > 0 else (xc + u2q))

        def k_piece(slot, ci):
            def f(anchor):
                kb[slot, zrows(D, 16, 16), 0:R] = anchor[0:16].astype(bf16)
                kprep(slot, ci, an_scr)
                add_fence(KLAG, _bits(an_scr[0, zrows(ci * (R // 2)), :]))
            return f

        def v_pieces(slot, ms, vps, dst):
            def mk(g, rb, e, fence):
                def f(anchor):
                    vb[slot, zrows(D, 16, 16), 0:R] = anchor[0:16].astype(bf16)
                    vprep(slot, ms, g, rb, e, dst)
                    if fence:
                        add_fence(KLAG, _bits(dst.bitcast(u32)[3 * e, g, zrows(rb * 8), :]))
                return f
            return [mk(g, rb, e, n % 4 == 3 or n == len(vps) - 1) for n, (g, rb, e) in enumerate(vps)]

        def stage(kslot, kcs, vslot, ms, vps, kgap=20, k0=8, mu=False):
            out = [[] for _ in range(NST)]
            for n, ci in enumerate(kcs):
                out[k0 + n * kgap].append(k_piece(kslot, ci))
            _spread(v_pieces(vslot, ms, vps, xn_w), out)
            if mu:
                out[44].append(mu_piece(vslot, ms))
            return out

        def weights(slot, u, hh):
            qc = qb[slot, :, pl.ds(u * W + hh * R, R)]
            return (qc[0:128], jnp.concatenate([qc[0:64], qc[128:192]], axis=0), qc[64:192])

        def trio(ws, s_ref, ci, hh):
            rows = pl.ds(ci * R // 2, R // 2)
            tok = take_fences()
            m3 = jnp.dot(lhs(a_scr[2, rows, :], tok), ws[2], preferred_element_type=f32)
            m1 = jnp.dot(lhs(a_scr[0, rows, :], tok), ws[0], preferred_element_type=f32)
            m2 = jnp.dot(lhs(a_scr[1, rows, :], tok), ws[1], preferred_element_type=f32)
            for _ in range(3):
                loads[loads.index(min(loads))] += R
            sa = (m1 + m3) * c
            sb = (m2 + m3) * c
            s_ref[hh, 2 * ci] = sa
            s_ref[hh, 2 * ci + 1] = sb
            t = jnp.maximum(sa, sb).reshape(R // 8, 8, R).max(axis=0)
            add_fence(SLAG, _bits(s_ref[0, 0, zrows(), :]) | _bits(t))
            return t, m3

        def row_shift(ts):
            m = jnp.max(_tree(ts, jnp.maximum), axis=0, keepdims=True)
            n2 = jnp.sum(_tree([jnp.exp2((t - m) * 2.0) for t in ts], jnp.add), axis=0, keepdims=True)
            return _bits(jnp.broadcast_to(m + jnp.log2(n2) * 0.5, (8, R)))

        def sm_slab(par, idx, m8, l, anchors):
            g, b = divmod(idx, SPG)
            rows = pl.ds(b * SLAB, SLAB)
            yrows = pl.ds(g * R + b * SLAB, SLAB)

            def mk_exp(anchor, qs):
                tk = _bits(anchor) & zero["v"]
                mm = {qq: lax.bitcast_convert_type(m8[qq] | tk, f32) for qq in qs}
                mm = {qq: jnp.concatenate([x, x], axis=0) for qq, x in mm.items()}
                return lambda kk, qq: jnp.exp2(sbufs[par][qq, 4 * g + kk, rows, :] - mm[qq])

            def put(r, x):
                ybufs[par][r, yrows, :] = x.astype(bf16)

            def diff(kk, qq, pkq, pqk):
                put(3 * PAIRS.index((kk, qq)) + 2, pkq - pqk)

            def single(kk, qq, p):
                if kk < qq:
                    put(3 * PAIRS.index((kk, qq)), p)
                else:
                    put(3 * PAIRS.index((qq, kk)) + 1, p)

            uc = {}
            ur = {}
            for n, (i, j) in enumerate(((0, 3), (1, 2))):
                ex = mk_exp(anchors[n], (i, j))
                pii, pjj, pij, pji = ex(i, i), ex(j, j), ex(i, j), ex(j, i)
                single(i, j, pij)
                single(j, i, pji)
                diff(i, j, pij, pji)
                uc[i] = pii + pji
                uc[j] = pjj + pij
                ur[i] = pii + pij
                ur[j] = pjj + pji
            keep = {}
            l = list(l)
            for n, (rs, cs) in enumerate((((0, 3), (1, 2)), ((1, 2), (0, 3)))):
                ex = mk_exp(anchors[2 + n], cs)
                p = {(kk, qq): ex(kk, qq) for kk in rs for qq in cs}
                for (kk, qq), x in p.items():
                    single(kk, qq, x)
                for kk in rs:
                    put(19 + 2 * kk, ur[kk] - (p[(kk, cs[0])] + p[(kk, cs[1])]))
                for qq in cs:
                    vc = p[(rs[0], qq)] + p[(rs[1], qq)]
                    put(18 + 2 * qq, uc[qq] - vc)
                    tot = uc[qq] + vc
                    tot = tot[0:8] + tot[8:16]
                    l[qq] = tot if l[qq] is None else l[qq] + tot
                if n == 0:
                    keep = p
                else:
                    for (kk, qq), x in p.items():
                        if kk < qq:
                            diff(kk, qq, x, keep[(qq, kk)])
                        else:
                            diff(qq, kk, keep[(qq, kk)], x)
            return l

        def y_fence(par, l, lag):
            tok = _bits(ybufs[par][0, zrows(0, 8, 16), :].astype(f32))
            add_fence(lag, _tree([tok] + [_bits(x) for x in l], jnp.bitwise_or))

        def queue_pv(par, swap_x):
            ms = {}

            def mk(i, j):
                def f(tok, even=False):
                    yy = pltpu.bitcast(ybufs[par].bitcast(u32)[i, pl.ds(j * R // 2, R // 2), :], bf16)
                    xx = lhs(x_scr[i, j], tok)
                    if even:
                        assert loads[0] == loads[1] == loads[2] == loads[3] - hd // 3
                        o = jnp.concatenate(
                            [jnp.dot(xx[a:a + hd // 3], yy, preferred_element_type=f32)
                             for a in range(0, hd, hd // 3)], axis=0)
                    else:
                        o = jnp.dot(xx, yy, preferred_element_type=f32)
                    ms[i] = o if j == 0 else ms[i] + o
                    loads[loads.index(min(loads))] += hd
                    if swap_x and j % 2 == 1:
                        xn_scr[NP, 0, zrows(), :] = lax.bitcast_convert_type(o[0:8], u32)
                        for jj in (j - 1, j):
                            x_scr[i, jj] = xn_scr[i, jj]
                    if j == NG - 1:
                        mbufs[par][i] = ms[i]
                        add_fence(CLAG, _bits(mbufs[par][i, zrows(), :]))
                    return o
                return f

            for i in range(NP):
                for j in range(NG):
                    pend.append(mk(i, j))

        def fin_pieces(fin, l_fin):
            slot, u, par, ms = fin
            m_ref = mbufs[par]
            rls = {}

            def mk(qq, rb):
                def f(anchor):
                    if anchor is not None:
                        m_ref[NP, zrows(), :] = anchor[0:8]
                    if qq not in rls:
                        rls[qq] = 1.0 / jnp.sum(l_fin[qq], axis=0, keepdims=True)

                    def prod(r):
                        return m_ref[r, pl.ds(rb * 16, 16), :]

                    gq = prod(19 + 2 * qq)
                    oth = []
                    for e, (i, j) in enumerate(PAIRS):
                        b = BS[(i, j)]
                        if qq == j:
                            oth.append((i, prod(3 * e), 1.0))
                            gq = gq - (prod(3 * e + 1) + prod(3 * e + 2))
                        elif qq == i:
                            d = prod(3 * e) - prod(3 * e + 2)
                            gq = (gq + d) if b > 0 else (gq - d)
                            oth.append((j, prod(3 * e + 1), -b))
                    c1 = prod(18 + 2 * qq) - gq * T[qq]
                    c2 = gq
                    for kk, gv, sg in oth:
                        c1 = c1 - gv * (T[kk] * sg)
                        c2 = (c2 + gv) if sg > 0 else (c2 - gv)
                    cols = pl.ds(u * W + qq * R, R)
                    for r0, cc in ((rb * 16, c1), (hd + rb * 16, c2)):
                        outb[slot, pl.ds(r0, 16), cols] = (cc * rls[qq] + mu_scr[ms, pl.ds(r0, 16), :]).astype(bf16)
                    if anchor is not None and rb % 3 == 2:
                        add_fence(KLAG, _bits(outb[slot, zrows(rb * 16, 8, 16), cols].astype(f32)))
                return f
            return [mk(qq, rb) for qq in range(NQ) for rb in range(NRB)]

        def step(qk, sm, pv, fin, st, swap_a=False, swap_x=False, final=0, stg=None, qx=(), mid=None):
            m_sm, l_pv, l_fin = st
            if pv is not None:
                queue_pv(pv, swap_x)
            stg = stg or [[] for _ in range(NST)]
            qs = [[] for _ in range(NQ * NC)]
            _spread(list(qx), qs[:NQ * NC - 2])
            if fin is not None:
                fp = fin_pieces(fin, l_fin)
                if pv is None:
                    for piece in fp:
                        piece(None)
                elif qk is not None:
                    _spread(fp, qs[2:2 + len(fp)])
                else:
                    if sm is not None:
                        stg += [[] for _ in range(100 - len(stg))]
                    _spread(fp, stg)
            l = [None] * NQ
            shifts = []
            ns = 0
            if qk is not None:
                for hh in range(NQ):
                    ws = weights(qk[0], qk[1], hh)
                    ts = []
                    for ci in range(NC):
                        clock[0] += 1
                        t, m3 = trio(ws, sbufs[qk[2]], ci, hh)
                        ts.append(t)
                        if swap_a and hh == NQ - 1:
                            rows = pl.ds(ci * R // 2, R // 2)
                            a_scr[:, rows, :] = an_scr[:, rows, :]
                        while pend and loads[3] < loads[0]:
                            pend.pop(0)(None)
                        l = sm_slab(sm, ns, m_sm, l, [m3[i * 24:i * 24 + 8] for i in range(4)])
                        y_fence(sm, l, YLAG)
                        for n, piece in enumerate(qs[ns]):
                            r0 = 112 if len(qs[ns]) == 1 else (n * 112 // (len(qs[ns]) - 1)) // 8 * 8
                            piece(m3[r0:r0 + 16])
                        ns += 1
                    shifts.append(row_shift(ts))
            if mid is not None:
                mid()
            n = 0
            recent = []
            while pend:
                if (not final and len(pend) <= 3
                        and loads[0] == loads[1] == loads[2] and loads[3] >= loads[0]):
                    break
                if n % 4 == 0:
                    clock[0] += 1
                n += 1
                tile = pend.pop(0)
                o = tile(take_fences(flush=(final and len(pend) == 1)), final == 2 and not pend)
                if stg:
                    for piece in stg.pop(0):
                        piece(o)
                if sm is not None and ns < NG * SPG:
                    recent.append(o)
                    if len(recent) == 3:
                        l = sm_slab(sm, ns, m_sm, l,
                                    [recent[0][0:8], recent[1][16:24], recent[2][32:40], recent[2][56:64]])
                        ns += 1
                        recent = []
                        y_fence(sm, l, ELAG)
            assert not any(stg) and (sm is None or ns == NG * SPG)
            return (tuple(shifts) if qk is not None else None), (tuple(l) if sm is not None else None), l_pv

        vall = [(g, rb, e) for g in range(NG) for rb in range(NRB) for e in range(7)]
        nv = len(vall) // 3

        def q0_copy(a, b, sem):
            cs = pl.ds(a * W, (b - a) * W)
            return pltpu.make_async_copy(q_hbm.at[0, :, cs], qb.at[0, :, cs], p_sem.at[sem])

        def k0_copy(hf, sem):
            cs = pl.ds(hf * half, half)
            return pltpu.make_async_copy(k_hbm.at[0, :, cs], kb.at[0, pl.ds(0, D), cs], p_sem.at[sem])

        ck0a, ck0b = k0_copy(0, 0), k0_copy(1, 1)
        cq0, cq1, cq2 = q0_copy(0, 1, 2), q0_copy(1, 2, 3), q0_copy(2, 4, 4)
        for cp in (ck0a, cq0, ck0b, v_copy(0, 0), cq1, cq2, k_copy(1, 1), v_copy(1, 1)):
            cp.start()
        small = lax.fori_loop(0, 3, lambda i, acc: acc + i, jnp.int32(0))
        ck0a.wait()
        cq0.wait()
        new_block(small)
        wss = [weights(0, 0, hh) for hh in range(NQ)]
        tss = [[] for _ in range(NQ)]
        v0 = sorted(vall, key=lambda x: x[2])
        qs0 = [[] for _ in range(NC * NQ // 2)]
        _spread(v_pieces(0, 0, v0[:104], x_w), qs0)
        for ci in range(NC):
            if ci == NC // 2:
                ck0b.wait()
                v_copy(0, 0).wait()
                cq1.wait()
                new_block(small)
                mu_piece(0, 0)(None)
            kprep(0, ci, a_scr)
            for hh in range(NQ):
                clock[0] += 1
                t, m3 = trio(wss[hh], sbufs[0], ci, hh)
                tss[hh].append(t)
                if ci >= NC // 2:
                    for n, piece in enumerate(qs0.pop(0)):
                        piece(m3[(n * 24) % 112:(n * 24) % 112 + 16])
        st = (tuple(row_shift(t) for t in tss), None, None)
        st = step((0, 1, 1), 0, None, None, st)
        cq2.wait()
        k_copy(1, 1).wait()
        v_copy(1, 1).wait()
        q_copy(1, 1).start()
        k_copy(2, 0).start()
        new_block(small)
        mu_piece(1, 1)(None)
        st = step((0, 2, 0), 1, 0, None, st, final=2, stg=stage(1, range(NC), 1, 1, vall[:nv], 6, 0),
                  qx=v_pieces(0, 0, v0[104:], x_w), mid=lambda: v_copy(2, 0).start())

        def head(h, st):
            cur = h & 1
            nx = 1 - cur
            new_block(h)
            mu0, mu1, mu2 = h & 3, (h + 1) & 3, (h + 2) & 3
            q_copy(0, nx).wait()
            k_copy(0, cur).wait()
            v_copy(0, cur).wait()

            @pl.when(h > 1)
            def _():
                out_copy(h - 2, cur).wait()

            @pl.when(h > 0)
            def _():
                out_copy(h - 1, nx).start()

            k_copy(jnp.minimum(h + 3, H - 1), nx).start()
            add_fence(3, _bits(kb[cur, zrows(0, 8, 16), 0:R].astype(f32)))
            st = step((cur, 3, 1), 0, 1, (cur, 0, 0, mu0), st, swap_a=True,
                      stg=stage(cur, [0, 1], nx, mu1, vall[nv:2 * nv]))
            q_copy(jnp.minimum(h + 2, H - 1), cur).start()
            st = step((nx, 0, 0), 1, 0, (cur, 1, 1, mu0), st, stg=stage(cur, [2, 3], nx, mu1, vall[2 * nv:]))
            v_copy(jnp.minimum(h + 3, H - 1), nx).start()
            add_fence(12, _bits(vb[cur, zrows(0, 8, 16), 0:R].astype(f32)))
            st = step((nx, 1, 1), 0, 1, (cur, 2, 0, mu0), st, swap_x=True,
                      stg=stage(cur, [4, 5, 6, 7], cur, mu2, [], 12, 0, mu=True))
            return step((nx, 2, 0), 1, 0, (cur, 3, 1, mu0), st, final=2, stg=stage(cur, [], cur, mu2, vall[:nv]))

        st = lax.fori_loop(0, H - 1, head, st)

        last = (H - 1) % 2
        new_block(small)

        def last_copy(a, b, sem):
            cs = pl.ds(a * W, (b - a) * W)
            return pltpu.make_async_copy(outb.at[last, :, cs], o_hbm.at[H - 1, :, cs], p_sem.at[sem])

        e1, e2 = last_copy(0, 3, 1), last_copy(3, 4, 2)
        out_copy(H - 3, last).wait()
        out_copy(H - 2, 1 - last).start()
        st = step((last, 3, 1), 0, 1, (last, 0, 0, (H - 1) & 3), st, final=1)
        st = step(None, 1, 0, (last, 1, 1, (H - 1) & 3), st, final=1)
        st = step(None, None, 1, (last, 2, 0, (H - 1) & 3), st, final=1)
        e1.start()
        step(None, None, None, (last, 3, 1, (H - 1) & 3), st, final=1)
        e2.start()
        q_copy(0, 1 - last).wait()
        k_copy(0, last).wait()
        v_copy(0, last).wait()
        out_copy(H - 2, 1 - last).wait()
        e1.wait()
        e2.wait()

    ot = pl.pallas_call(
        body,
        in_specs=[pl.BlockSpec(memory_space=pl.ANY)] * 3,
        out_specs=pl.BlockSpec(memory_space=pl.ANY),
        out_shape=jax.ShapeDtypeStruct((H, D, S), bf16),
        scratch_shapes=[
            pltpu.VMEM((2, D, S), bf16),
            pltpu.VMEM((2, D + 16, S), bf16),
            pltpu.VMEM((2, D + 16, S), bf16),
            pltpu.VMEM((2, D, S), bf16),
            pltpu.VMEM((3, half // 2, R), u32),
            pltpu.VMEM((NP, NG, hd, R), bf16),
            pltpu.VMEM((3, half // 2, R), u32),
            pltpu.VMEM((NP + 1, NG, hd, R), bf16),
            pltpu.VMEM((NQ, 2 * NC, R, R), f32),
            pltpu.VMEM((NQ, 2 * NC, R, R), f32),
            pltpu.VMEM((NP, NG * R + 16, R), bf16),
            pltpu.VMEM((NP, NG * R + 16, R), bf16),
            pltpu.VMEM((NP + 1, hd, R), f32),
            pltpu.VMEM((NP + 1, hd, R), f32),
            pltpu.VMEM((4, D, R), f32),
            pltpu.SemaphoreType.DMA((2,)),
            pltpu.SemaphoreType.DMA((2,)),
            pltpu.SemaphoreType.DMA((2,)),
            pltpu.SemaphoreType.DMA((2,)),
            pltpu.SemaphoreType.DMA((5,)),
        ],
        compiler_params=pltpu.CompilerParams(vmem_limit_bytes=100 * 1024 * 1024),
    )(qt, kt, vt)
    return jnp.swapaxes(ot.reshape(B, NH, D, S), 2, 3)
```
